```python
import os as _os
_os.environ.setdefault("JAX_PLATFORMS", "cpu")
import jax
import jax.numpy as jnp

def _softmax(x, axis=-1):
    return jax.nn.softmax(x, axis=axis)
def _gelu(x):
    return jax.nn.gelu(x, approximate=True)
def _silu(x):
    return jax.nn.silu(x)
def _sigmoid(x):
    return jax.nn.sigmoid(x)
def _layernorm(x, axis=-1, eps=1e-5):
    m = jnp.mean(x, axis=axis, keepdims=True)
    v = jnp.var(x, axis=axis, keepdims=True)
    return (x - m) / jnp.sqrt(v + eps)
def _scatter_add(tgt, idx, src, axis=0):
    return tgt.at[idx].add(src)
def _segment_sum(src, seg, n):
    return jax.ops.segment_sum(src, seg, n)
class _Rng:
    def __init__(self, key):
        self._k = key
    def _next(self):
        self._k, sub = jax.random.split(self._k)
        return sub
    def normal(self, shape):
        return jax.random.normal(self._next(), shape, dtype=jnp.bfloat16)
    def randint(self, lo, hi, shape):
        return jax.random.randint(self._next(), shape, lo, hi, dtype=jnp.int32)
    def uniform(self, shape, lo=0.0, hi=1.0):
        return jax.random.uniform(self._next(), shape, jnp.bfloat16, lo, hi)
    def permutation(self, n):
        return jax.random.permutation(self._next(), n)


kernel_name = 'gated_mix__spectral_gfnet__dense_activation_silu__prompt'

def setup_inputs():
    _rng = _Rng(jax.random.key(int.from_bytes(__import__("os").urandom(4), "little")))
    _w = (lambda a: (lambda t: t.astype(jnp.bfloat16) if jnp.issubdtype(t.dtype, jnp.floating) else t)(jnp.asarray(a)))
    def _A_setup():
        B, S, D = 1, 2048, 512
        Df = D // 2 + 1
        return {
            "x": _w((lambda *s: _rng.normal(s) * 0.05)(B, S, D)),
            "w_r": _w((lambda *s: _rng.normal(s) * 0.05)(S, Df) * 0.02),
            "w_i": _w((lambda *s: _rng.normal(s) * 0.05)(S, Df) * 0.02),
        }
    _A_in = _A_setup()

    def _B_setup():
        B, S, D, F = 1, 2048, 512, 1376
        return {
            "x": _w((lambda *s: _rng.normal(s) * 0.05)(B, S, D)),
            "w1": _w((lambda *s: _rng.normal(s) * 0.05)(D, F) * (D ** -0.5)),
            "w2": _w((lambda *s: _rng.normal(s) * 0.05)(F, D) * (F ** -0.5)),
        }
    _B_in = _B_setup()

    return {
        "A_x": _A_in["x"],
        "A_w_r": _A_in["w_r"],
        "A_w_i": _A_in["w_i"],
        "B_x": _B_in["x"],
        "B_w1": _B_in["w1"],
        "B_w2": _B_in["w2"],
        "gate_w": _w((lambda *s: _rng.normal(s) * 0.05)(512) * 16.0),
    }

def reference(A_x, A_w_r, A_w_i, B_x, B_w1, B_w2, gate_w):
    def _A_ref(x, w_r, w_i):
        B, S, D = x.shape
        X = (lambda x, axes=(-2,-1): jnp.fft.rfft2(x.astype(jnp.float32), axes=axes))(x, axes=(-2, -1))
        W = w_r + 1j * w_i
        X = X * W
        y = (lambda x, s, axes=(-2,-1): jnp.fft.irfft2(x, s=s, axes=axes).astype(jnp.bfloat16))(X, (S, D), axes=(-2, -1))
        return y

    def _B_ref(x, w1, w2):
        h = jnp.einsum("bsd,df->bsf", x, w1)
        h = _silu(h)
        out = jnp.einsum("bsf,fd->bsd", h, w2)
        return out

    x = A_x
    g = _sigmoid((x * gate_w).sum(-1, keepdims=True))
    a = _A_ref(x, A_w_r, A_w_i)
    b = _B_ref(x, B_w1, B_w2)
    return g * a + (1 - g) * b
```

```python
import functools
import numpy as np
import jax
import jax.numpy as jnp
from jax import lax
import jax.experimental.pallas as pl
import jax.experimental.pallas.tpu as pltpu

S, D, F = 2048, 512, 1376
FP = 1408
NF = 11
NT = (((1,), (1,)), ((), ()))
AS = 20
LAG = 1
AT = AS * 128
F32 = jnp.float32
BF16 = jnp.bfloat16
U32 = jnp.uint32

O_LD0, O_LD2, O_LD1, O_RD0, O_RD2, O_RD1, O_J, O_END = 0, 72, 136, 392, 456, 520, 776, 840


def _pack_rows(a):
    f = np.ascontiguousarray(a, dtype=np.float32)
    u = f.view(np.uint32).astype(np.uint64)
    b = ((u + 0x7FFF + ((u >> 16) & 1)) >> 16).astype(np.uint32)
    return (b[..., 0::2, :] | (b[..., 1::2, :] << 16)).astype(np.uint32)


def _consts():
    n2 = np.arange(128)
    j = np.arange(64)
    ld0 = np.zeros((144, 128))
    th = 2 * np.pi * np.outer(4 * j, n2) / 512
    ld0[0:64] = np.cos(th)
    ld0[64:128] = -np.sin(th)
    ld0[128] = np.cos(np.pi * n2)
    ld2 = np.zeros((128, 128))
    th = 2 * np.pi * np.outer(4 * j + 2, n2) / 512
    ld2[0:64] = np.cos(th)
    ld2[64:128] = -np.sin(th)
    i = np.arange(128)
    th = 2 * np.pi * np.outer(2 * i + 1, n2) / 512
    sg = np.where(i % 2 == 0, -1.0, 1.0)[:, None]
    ld1 = np.zeros((256, 256))
    ld1[0:128, 0:128] = np.cos(th)
    ld1[0:128, 128:256] = sg * np.sin(th)
    ld1[128:256, 0:128] = -np.sin(th)
    ld1[128:256, 128:256] = sg * np.cos(th)
    sc = 2.0 / (S * D)
    rd0 = np.zeros((128, 128))
    rd0[0::2] = ld0[0:64] * sc
    rd0[1::2] = ld0[64:128] * sc
    rd0[0] = ld0[0] * sc / 4
    rd0[1] = ld0[128] * sc / 4
    rd2 = np.zeros((128, 128))
    rd2[1::2] = ld2[0:64] * sc
    rd2[(2 * j + 2) % 128] = ld2[64:128] * sc
    rd1 = ld1 * sc
    e = np.arange(64)
    kl = np.arange(64)
    g = np.zeros((16, 2, 128, 128))
    for s_lo in range(16):
        for kb in range(2):
            th = -2 * np.pi * np.outer(s_lo + 16 * e, 2 * kl + kb) / S
            gr, gi = np.cos(th), np.sin(th)
            if kb == 0:
                rr, ri = slice(0, 64), slice(64, 128)
                cr, ci = 2 * kl, 2 * kl + 1
            else:
                rr, ri = slice(64, 128), slice(0, 64)
                cr, ci = 2 * kl + 1, (2 * kl + 2) % 128
            m = np.zeros((128, 128))
            m[rr, cr] = gr
            m[rr, ci] = gi
            m[ri, cr] = -gi
            m[ri, ci] = gr
            g[s_lo, kb] = m
    jrev = np.zeros((128, 128))
    jrev[np.arange(128), 127 - np.arange(128)] = 1.0
    perm = np.concatenate([np.arange(0, 128, 2), np.arange(1, 128, 2)])
    ld1 = ld1[np.concatenate([perm, 128 + perm])]
    small = np.concatenate([ld0, ld2, ld1[:, 0:128], ld1[:, 128:256], rd0, rd2,
                            rd1[:, 0:128], rd1[:, 128:256], jrev], axis=0)
    return _pack_rows(small), _pack_rows(g.reshape(32, 128, 128))


def _dft4(z, inv):
    (ar, ai), (br, bi), (cr, ci), (dr, di) = z
    s0r, s0i = ar + cr, ai + ci
    s1r, s1i = ar - cr, ai - ci
    s2r, s2i = br + dr, bi + di
    s3r, s3i = br - dr, bi - di
    y0 = (s0r + s2r, s0i + s2i)
    y2 = (s0r - s2r, s0i - s2i)
    if not inv:
        y1 = (s1r + s3i, s1i - s3r)
        y3 = (s1r - s3i, s1i + s3r)
    else:
        y1 = (s1r - s3i, s1i + s3r)
        y3 = (s1r + s3i, s1i - s3r)
    return [y0, y1, y2, y3]


def _tw16(z, ex, inv):
    r, i = z
    ex = ex % 16
    if ex == 0:
        return z
    sgn = 1.0 if inv else -1.0
    if ex == 4:
        return (-i, r) if inv else (i, -r)
    c = float(np.cos(2 * np.pi * ex / 16))
    s = sgn * float(np.sin(2 * np.pi * ex / 16))
    if ex in (2, 6):
        h = float(np.sqrt(0.5))
        if c > 0 and s > 0:
            return ((r - i) * h, (r + i) * h)
        if c > 0 and s < 0:
            return ((r + i) * h, (i - r) * h)
        if c < 0 and s > 0:
            return ((r + i) * (-h), (r - i) * h)
        return ((i - r) * h, (r + i) * (-h))
    return (r * c - i * s, r * s + i * c)


def _dft16(z, inv):
    a = [None] * 16
    for n2 in range(4):
        y = _dft4([z[4 * n1 + n2] for n1 in range(4)], inv)
        for k1 in range(4):
            a[4 * k1 + n2] = _tw16(y[k1], k1 * n2, inv)
    out = [None] * 16
    for k1 in range(4):
        y = _dft4([a[4 * k1 + n2] for n2 in range(4)], inv)
        for k2 in range(4):
            out[k1 + 4 * k2] = y[k2]
    return out


def _unpack(w, idx):
    return pltpu.unpack_elementwise(w, index=idx, packed_dtype=BF16, unpacked_dtype=F32)


def _bf(w):
    return pltpu.bitcast(w, BF16)


def _u32(v):
    return pltpu.bitcast(v, U32)


def _kernel(one_ref, x_hbm, wr_hbm, wi_hbm, w1_hbm, w2_hbm, gw_hbm, sm_hbm, g_hbm,
            o_hbm,
            xs, wrs, wis, nyq_r, nyq_i, w1s, w2s, gws, sm, gm,
            u_ref, t_ref, v_ref, a_ref, sp_ref, act, gate, os_, sem):
    lane = lax.broadcasted_iota(jnp.int32, (1, 128), 1)
    lo_half = lane < 64
    even = (lane % 2) == 0

    xb, w1b, w2b = xs.bitcast(BF16), w1s.bitcast(BF16), w2s.bitcast(BF16)
    wrb, wib = wrs.bitcast(BF16), wis.bitcast(BF16)
    uw, vw, actw = u_ref.bitcast(U32), v_ref.bitcast(U32), act.bitcast(U32)

    def pk(lo, hi):
        return pltpu.pack_elementwise([lo, hi], packed_dtype=BF16).astype(U32)

    nsem = [0]

    def group(pairs):
        k = nsem[0]
        nsem[0] += 1
        return [pltpu.make_async_copy(s, d, sem.at[k]) for s, d in pairs]

    def start(cps):
        for c in cps:
            c.start()

    def wait(cps):
        for c in cps:
            c.wait()

    def w1_group(f0, f1):
        return group([(w1_hbm.at[pl.ds(f0, f1 - f0), pl.ds(128 * t, 128)],
                       w1b.at[t, pl.ds(f0, f1 - f0), :]) for t in range(4)])

    def x_group(i):
        return group([(x_hbm.at[pl.ds(1024 * c + 256 * i, 256), pl.ds(128 * t, 128)],
                       xb.at[pl.ds(S * t + 1024 * c + 256 * i, 256), :])
                      for c in range(2) for t in range(4)])

    d_w1a = w1_group(0, 256)
    d_x = [x_group(i) for i in range(4)]
    d_sm = group([(sm_hbm, sm), (gw_hbm, gws)])
    d_w1b = w1_group(256, 384)
    d_g = group([(g_hbm, gm)])
    d_w = group([(wr_hbm.at[pl.ds(0, 256), pl.ds(128 * t, 128)], wrb.at[t]) for t in range(16)]
                + [(wi_hbm.at[pl.ds(0, 256), pl.ds(128 * t, 128)], wib.at[t]) for t in range(16)]
                + [(wr_hbm.at[pl.ds(256, 1), :], nyq_r), (wi_hbm.at[pl.ds(256, 1), :], nyq_i)])
    d_w1c = w1_group(384, F)
    d_w2 = group([(w2_hbm.at[:, pl.ds(128 * t, 128)], w2b.at[t, pl.ds(0, F), :]) for t in range(4)])

    for d in [d_w1a] + d_x + [d_sm, d_w1b, d_g, d_w1c, d_w, d_w2]:
        start(d)

    for t in range(4):
        w2s[t, F // 2:FP // 2, :] = jnp.zeros(((FP - F) // 2, 128), U32)

    def mm1(ranges, nts):
        x = jnp.concatenate(
            [jnp.concatenate([_bf(xs[1024 * t + r0 // 2:1024 * t + r1 // 2, :]) for t in range(4)], axis=1)
             for r0, r1 in ranges], axis=0)
        for nt in nts:
            w = jnp.concatenate([_bf(w1s[t, 64 * nt:64 * (nt + 1), :]) for t in range(4)], axis=1)
            h = lax.dot_general(x, w, NT, preferred_element_type=F32)
            hh = 0.5 * h
            th = jnp.tanh(hh)
            af = hh + hh * th
            a = af.astype(BF16)
            if nt == NF - 1:
                g = 0.5 * th[:, F - 1280:F - 1279] + 0.5
                gb = jnp.broadcast_to(g, (g.shape[0], 128))
            off = 0
            for r0, r1 in ranges:
                act[nt, r0:r1, :] = a[off:off + r1 - r0]
                if nt == NF - 1:
                    gate[r0:r1, :] = gb[off:off + r1 - r0]
                off += r1 - r0
        return af

    def f1(i):
        base = 128 * i
        for p in range(8):
            w0 = [xs[pl.ds(1024 * t + base + p, 16, stride=8), :] for t in range(4)]
            w1 = [xs[pl.ds(1024 * t + 512 + base + p, 16, stride=8), :] for t in range(4)]
            for h in range(2):
                s_lo = 2 * p + h
                x0 = [_unpack(w, h) for w in w0]
                x1 = [_unpack(w, h) for w in w1]
                for kb, z in enumerate(([a + b for a, b in zip(x0, x1)], [a - b for a, b in zip(x0, x1)])):
                    y0, y1, y2, y3 = z
                    a0, a1 = y0 + y2, y1 + y3
                    for t, uu in enumerate((a0 + a1, a0 - a1, y0 - y2, y1 - y3)):
                        u_ref[s_lo, t, 64 * kb + 16 * i:64 * kb + 16 * i + 16, :] = uu.astype(BF16)

    def phase_a1(s_lo):
        u = [_bf(uw[s_lo, t]) for t in range(4)]
        ld0 = _bf(sm[O_LD0:O_LD2, :])
        ld2 = _bf(sm[O_LD2:O_LD1, :])
        ld1 = jnp.concatenate([_bf(sm[O_LD1:O_LD1 + 128, :]), _bf(sm[O_LD1 + 128:O_RD0, :])], axis=1)
        o0 = lax.dot_general(ld0, u[0], NT, preferred_element_type=F32)
        o2 = lax.dot_general(ld2, u[1], NT, preferred_element_type=F32)
        o1 = lax.dot_general(ld1, jnp.concatenate([u[2], u[3]], axis=1), NT, preferred_element_type=F32)
        r_e = pk(o0[0:64], o2[0:64])
        i_e = pk(o0[64:128], o2[64:128])
        r_o = pk(o1[0:64], o1[64:128])
        i_o = pk(o1[128:192], o1[192:256])
        r_n = pk(o0[128:136], o0[136:144])
        zero = jnp.zeros_like(r_n)
        r = jnp.concatenate([r_e, r_o], axis=0)
        t = pltpu.roll(jnp.concatenate([i_e, i_o], axis=0), 64, 1)
        la = _bf(jnp.concatenate([jnp.where(lo_half, r, t), jnp.where(lo_half, r_n, zero)], axis=0))
        lb = _bf(jnp.concatenate([jnp.where(lo_half, t, r), jnp.where(lo_half, zero, r_n)], axis=0))
        return la, lb

    def phase_a2(s_lo, la, lb):
        oa = jnp.dot(la, _bf(gm[2 * s_lo]), preferred_element_type=F32)[0:264]
        ob_ = jnp.dot(lb, _bf(gm[2 * s_lo + 1]), preferred_element_type=F32)[0:264]
        t_ref[s_lo, 0, 0:264, :] = jnp.where(even, oa, ob_)
        t_ref[s_lo, 1, 0:264, :] = pltpu.roll(jnp.where(even, ob_, oa), 127, 1)

    row8 = lax.broadcasted_iota(jnp.int32, (8, 128), 0)

    def special():
        row = lax.broadcasted_iota(jnp.int32, (16, S), 0)

        def rowcat(ref):
            return jnp.broadcast_to(
                jnp.concatenate([_unpack(ref[t, 0:1, :], 0) for t in range(16)], axis=1), (16, S))
        q = jnp.where(row == 0, rowcat(wrs),
            jnp.where(row == 1, rowcat(wis),
            jnp.where(row == 2, jnp.broadcast_to(nyq_r[...].astype(F32), (16, S)),
            jnp.where(row == 3, jnp.broadcast_to(nyq_i[...].astype(F32), (16, S)), 0.0))))
        qb = q.astype(BF16)
        stacked = jnp.concatenate([qb[:, 128 * (15 - t):128 * (16 - t)] for t in range(16)], axis=0)
        rv = jnp.dot(stacked, _bf(sm[O_J:O_END, :]), preferred_element_type=F32)
        rev = jnp.concatenate([rv[16 * t:16 * t + 8] for t in range(16)], axis=1)
        mir = pltpu.roll(rev, 1, 1)
        sgn = jnp.where((lax.broadcasted_iota(jnp.int32, (8, S), 0) % 2) == 0, 1.0, -1.0)
        sp_ref[...] = q[0:8] + sgn * mir

    def ld(s, r0):
        return t_ref[s, 0, r0:r0 + 8, :], t_ref[s, 1, r0:r0 + 8, :]

    def st(s, r0, z):
        t_ref[s, 0, r0:r0 + 8, :] = z[0]
        t_ref[s, 1, r0:r0 + 8, :] = z[1]

    def sp_row(r, kt, other):
        return jnp.where(row8 == 0, jnp.broadcast_to(sp_ref[r:r + 1, 128 * kt:128 * (kt + 1)], (8, 128)), other)

    def p1(r0, n2):
        y = _dft4([ld(4 * n1 + n2, r0) for n1 in range(4)], False)
        for k1 in range(4):
            st(4 * k1 + n2, r0, _tw16(y[k1], k1 * n2, False))

    def p2(r0, k1):
        y = _dft4([ld(4 * k1 + n2, r0) for n2 in range(4)], False)
        u = []
        for k2 in range(4):
            kt = k1 + 4 * k2
            if r0 == 256:
                wr, wi = sp_row(2, kt, 0.0), sp_row(3, kt, 0.0)
            else:
                i8, h = r0 % 128, r0 // 128
                wr, wi = _unpack(wrs[kt, i8:i8 + 8, :], h), _unpack(wis[kt, i8:i8 + 8, :], h)
                if r0 == 0:
                    wr, wi = sp_row(0, kt, wr), sp_row(1, kt, wi)
            xr, xi = y[k2]
            ur, ui = xr * wr - xi * wi, xr * wi + xi * wr
            if r0 == 0:
                er, ei = ld(4 * k1 + k2, 256)
                ur, ui = ur - ei, ui + er
            u.append((ur, ui))
        if r0 == 256:
            for k2 in range(4):
                st(4 * k1 + k2, r0, u[k2])
            return
        y = _dft4(u, True)
        for n2 in range(4):
            st(4 * k1 + n2, r0, _tw16(y[n2], k1 * n2, True))

    def p3(r0, n2):
        y = _dft4([ld(4 * k1 + n2, r0) for k1 in range(4)], True)
        for n1 in range(4):
            v_ref[4 * n1 + n2, 0, r0:r0 + 8, :] = y[n1][0].astype(BF16)
            v_ref[4 * n1 + n2, 1, r0:r0 + 8, :] = y[n1][1].astype(BF16)

    def phase_c1(s_lo):
        vr = vw[s_lo, 0]
        t = pltpu.roll(vw[s_lo, 1], 1, 1)
        va = _bf(jnp.where(even, vr, t))
        vb = _bf(jnp.where(even, t, vr))
        za = lax.dot_general(_bf(gm[2 * s_lo]), va, NT, preferred_element_type=F32)
        zb = lax.dot_general(_bf(gm[2 * s_lo + 1]), vb, NT, preferred_element_type=F32)
        zr = pk(za[0:64] + zb[64:128], za[0:64] - zb[64:128])
        zi = pk(za[64:128] + zb[0:64], za[64:128] - zb[0:64])
        re = zr[:, 0:128]
        t = pltpu.roll(zi[:, 0:128], 1, 1)
        l0 = _bf(jnp.where(even, re, t))
        l2 = _bf(jnp.where(even, t, re))
        l1 = _bf(jnp.concatenate([zr[:, 128:256], zi[:, 128:256]], axis=1))
        return l0, l2, l1

    def phase_c2(s_lo, l0, l2, l1):
        rd1 = jnp.concatenate([_bf(sm[O_RD1:O_RD1 + 128, :]), _bf(sm[O_RD1 + 128:O_J, :])], axis=1)
        a0 = jnp.dot(l0, _bf(sm[O_RD0:O_RD2, :]), preferred_element_type=F32)
        a2 = jnp.dot(l2, _bf(sm[O_RD2:O_RD1, :]), preferred_element_type=F32)
        pq = jnp.dot(l1, rd1, preferred_element_type=F32)
        pp, qq = pq[:, 0:128], pq[:, 128:256]
        e0, e1 = a0 + a2, a0 - a2
        for t, y in enumerate([e0 + pp, e1 + qq, e0 - pp, e1 - qq]):
            a_ref[pl.ds(AT * t + s_lo, 128, stride=AS), :] = y

    def mm2(r0, r1):
        lhs = jnp.concatenate([_bf(actw[nt, r0 // 2:r1 // 2, :]) for nt in range(NF)], axis=1)
        w2 = jnp.concatenate([_bf(w2s[t]) for t in range(4)], axis=1)
        b = jnp.dot(lhs, w2, preferred_element_type=F32)
        g = gate[r0:r1, :]
        for t in range(4):
            bt = b[:, 128 * t:128 * (t + 1)]
            pos = [AT * t + AS * (2 * ((r % 1024) // 16) + r // 1024) for r in range(r0, r1, 16)]
            at = jnp.concatenate([a_ref[p:p + 16, :] for p in pos], axis=0)
            os_[t, r0:r1, :] = (bt + g * (at - bt)).astype(BF16)
        cps = group([(os_.at[t, pl.ds(r0, r1 - r0), :], o_hbm.at[pl.ds(r0, r1 - r0), pl.ds(128 * t, 128)])
                     for t in range(4)])
        start(cps)
        return cps

    nreg = [0]

    def region(fn):
        pl.when(one_ref[nreg[0]] == 1)(fn)
        nreg[0] += 1

    def r_f1():
        wait(d_w1a)
        for i in range(4):
            wait(d_x[i])
            mm1([(256 * i, 256 * i + 256), (1024 + 256 * i, 1024 + 256 * i + 256)], (0, 1))
            f1(i)

    z = one_ref[7] - 1

    def tok(v):
        t_ref[0, 0, pl.ds(264 + z, 8), :] = v

    def r_a():
        wait(d_sm)
        wait(d_w1b)
        wait(d_g)
        gw = gws[...].reshape(1, D).astype(F32)
        rowp = lax.broadcasted_iota(jnp.int32, (FP - F, D), 0)
        padv = _u32(jnp.where(rowp == 0, jnp.broadcast_to(gw, (FP - F, D)), 0.0).astype(BF16))
        for t in range(4):
            w1s[t, F // 2:FP // 2, :] = padv[:, 128 * t:128 * (t + 1)]
        pend = []
        for s_lo in range(16 + LAG):
            if s_lo < 16:
                pend.append(phase_a1(s_lo))
            else:
                q = s_lo - 16
                mm1([(512 * q, 512 * q + 512)], (2,))
            if s_lo >= LAG:
                phase_a2(s_lo - LAG, *pend[s_lo - LAG])
        for q in range(LAG, 4):
            mm1([(512 * q, 512 * q + 512)], (2,))
        wait(d_w1c)
        wait(d_w)
        special()

    def r_b():
        rgs = [256] + [8 * i for i in range(32)]
        slots = []
        for j in range(len(rgs) + 2):
            for a in range(4):
                job = []
                if j < len(rgs):
                    job.append((p1, rgs[j], a))
                if 1 <= j - 2 < len(rgs):
                    job.append((p3, rgs[j - 2], a))
                if job:
                    slots.append(job)
                if 0 <= j - 1 < len(rgs):
                    slots.append([(p2, rgs[j - 1], a)])
        units = [(q, nt) for nt in range(3, 10) for q in range(4)]
        total = len(units) * 512
        step = (total - 64) / len(slots)
        j = 0
        for k, (q, nt) in enumerate(units):
            af = mm1([(512 * q, 512 * q + 512)], (nt,))
            while j < len(slots) and int(j * step) < 512 * (k + 1):
                r = ((int(j * step) - 512 * k) // 8) * 8
                tok(af[r:r + 8])
                for fn, r0, a in slots[j]:
                    fn(r0, a)
                j += 1

    def r_c():
        pend = []
        for s_lo in range(16 + LAG):
            if s_lo < 16:
                pend.append(phase_c1(s_lo))
            else:
                q = s_lo - 16
                mm1([(512 * q, 512 * q + 512)], (10,))
            if s_lo >= LAG:
                phase_c2(s_lo - LAG, *pend[s_lo - LAG])
        for q in range(LAG, 4):
            mm1([(512 * q, 512 * q + 512)], (10,))

    def r_mm2():
        wait(d_w2)
        outs = []
        for r0, r1 in [(0, 512), (512, 1024), (1024, 1536), (1536, 1920), (1920, 2048)]:
            outs.append(mm2(r0, r1))
        for cps in outs:
            wait(cps)

    for r in (r_f1, r_a, r_b, r_c, r_mm2):
        region(r)


@jax.jit
def pallas_gated_mix__spectral_gfnet__dense_activation_silu__prompt_kernel(A_x, A_w_r, A_w_i, B_x, B_w1, B_w2, gate_w):
    small, g = _consts()
    out = pl.pallas_call(
        _kernel,
        out_shape=jax.ShapeDtypeStruct((S, D), BF16),
        in_specs=[pl.BlockSpec(memory_space=pltpu.SMEM)] + [pl.BlockSpec(memory_space=pl.ANY)] * 8,
        out_specs=pl.BlockSpec(memory_space=pl.ANY),
        scratch_shapes=[
            pltpu.VMEM((4 * S // 2, 128), U32),
            pltpu.VMEM((16, 128, 128), U32),
            pltpu.VMEM((16, 128, 128), U32),
            pltpu.VMEM((1, S), BF16),
            pltpu.VMEM((1, S), BF16),
            pltpu.VMEM((4, FP // 2, 128), U32),
            pltpu.VMEM((4, FP // 2, 128), U32),
            pltpu.VMEM((D,), BF16),
            pltpu.VMEM((O_END, 128), U32),
            pltpu.VMEM((32, 64, 128), U32),
            pltpu.VMEM((16, 4, 128, 128), BF16),
            pltpu.VMEM((16, 2, 272, 128), F32),
            pltpu.VMEM((16, 2, 256, 128), BF16),
            pltpu.VMEM((4 * AT, 128), F32),
            pltpu.VMEM((8, S), F32),
            pltpu.VMEM((NF, S, 128), BF16),
            pltpu.VMEM((S, 128), F32),
            pltpu.VMEM((4, S, 128), BF16),
            pltpu.SemaphoreType.DMA((16,)),
        ],
        compiler_params=pltpu.CompilerParams(vmem_limit_bytes=100 * 1024 * 1024),
    )(jnp.ones((8,), jnp.int32), A_x[0], A_w_r.T, A_w_i.T, B_w1.T, B_w2, gate_w, jnp.asarray(small), jnp.asarray(g))
    return out[None]
```

```python
import functools
import numpy as np
import jax
import jax.numpy as jnp
from jax import lax
import jax.experimental.pallas as pl
import jax.experimental.pallas.tpu as pltpu

S, D, F = 2048, 512, 1376
FP = 1408
NF = 11
NT = (((1,), (1,)), ((), ()))
AS = 20
LAG = 1
DA = 3
DC = 2
HQ = float(np.sqrt(0.5))
UB = 258
NE = 5
AT = AS * 128
F32 = jnp.float32
BF16 = jnp.bfloat16
U32 = jnp.uint32

O_LD0, O_LD2, O_LDA, O_LDB, O_RD0, O_RD2, O_RDA, O_RDB, O_J, O_END = 0, 72, 136, 200, 264, 328, 392, 456, 520, 584


def _pack_rows(a):
    f = np.ascontiguousarray(a, dtype=np.float32)
    u = f.view(np.uint32).astype(np.uint64)
    b = ((u + 0x7FFF + ((u >> 16) & 1)) >> 16).astype(np.uint32)
    return (b[..., 0::2, :] | (b[..., 1::2, :] << 16)).astype(np.uint32)


def _consts():
    n2 = np.arange(128)
    j = np.arange(64)
    ld0 = np.zeros((144, 128))
    th = 2 * np.pi * np.outer(4 * j, n2) / 512
    ld0[0:64] = np.cos(th)
    ld0[64:128] = -np.sin(th)
    ld0[128] = np.cos(np.pi * n2)
    ld2 = np.zeros((128, 128))
    th = 2 * np.pi * np.outer(4 * j + 2, n2) / 512
    ld2[0:64] = np.cos(th)
    ld2[64:128] = -np.sin(th)
    i = np.arange(128)
    th = 2 * np.pi * np.outer(2 * i + 1, n2) / 512
    sg = np.where(i % 2 == 0, -1.0, 1.0)[:, None]
    ld1 = np.zeros((256, 256))
    ld1[0:128, 0:128] = np.cos(th)
    ld1[0:128, 128:256] = sg * np.sin(th)
    ld1[128:256, 0:128] = -np.sin(th)
    ld1[128:256, 128:256] = sg * np.cos(th)
    sc = 2.0 / (S * D)
    rd0 = np.zeros((128, 128))
    rd0[0::2] = ld0[0:64] * sc
    rd0[1::2] = ld0[64:128] * sc
    rd0[0] = ld0[0] * sc / 4
    rd0[1] = ld0[128] * sc / 4
    rd2 = np.zeros((128, 128))
    rd2[1::2] = ld2[0:64] * sc
    rd2[(2 * j + 2) % 128] = ld2[64:128] * sc
    hq = np.sqrt(0.5)
    eye, n64 = np.eye(256), np.arange(64)
    p_, q_ = eye[:, 0:128], eye[:, 128:256]
    lo = (np.arange(128) < 64)[None, :]
    e_ = np.where(lo, p_, hq * (p_ + q_))
    c_ = np.where(lo, q_, hq * (p_ - q_))
    r_ = np.roll(c_, 64, axis=1)
    mm = np.concatenate([e_ + r_, e_ - r_], axis=1).T
    ldv = ld1 @ mm.T / 2
    cls_a = (i % 4 == 0) | (i % 4 == 3)
    assert np.abs(ldv[np.concatenate([cls_a, cls_a])][:, 128:]).max() < 1e-9
    assert np.abs(ldv[np.concatenate([~cls_a, ~cls_a])][:, :128]).max() < 1e-9
    sg_ = np.arange(64)
    ia = np.where(sg_ % 2 == 0, 2 * sg_, 2 * sg_ + 1)
    ib = np.where(sg_ % 2 == 0, 2 * sg_ + 1, 2 * sg_)
    lda = np.concatenate([ldv[ia, :128], ldv[128 + ia, :128]], axis=0)
    ldb = np.concatenate([ldv[ib, 128:], ldv[128 + ib, 128:]], axis=0)
    rda, rdb = np.zeros((128, 128)), np.zeros((128, 128))
    ia_, ib_ = i[cls_a], i[~cls_a]
    rda[ia_] = ldv[ia_, :128] * sc
    rda[(ia_ + 2) % 128] = ldv[128 + ia_, :128] * sc
    rdb[ib_] = ldv[ib_, 128:] * sc
    rdb[(ib_ + 2) % 128] = ldv[128 + ib_, 128:] * sc
    e = np.arange(64)
    kl = np.arange(64)
    g = np.zeros((16, 2, 128, 128))
    for s_lo in range(16):
        for kb in range(2):
            th = -2 * np.pi * np.outer(s_lo + 16 * e, 2 * kl + kb) / S
            gr, gi = np.cos(th), np.sin(th)
            if kb == 0:
                rr, ri = slice(0, 64), slice(64, 128)
                cr, ci = 2 * kl, 2 * kl + 1
            else:
                rr, ri = slice(64, 128), slice(0, 64)
                cr, ci = 2 * kl + 1, (2 * kl + 2) % 128
            m = np.zeros((128, 128))
            m[rr, cr] = gr
            m[rr, ci] = gi
            m[ri, cr] = -gi
            m[ri, ci] = gr
            g[s_lo, kb] = m
    jrev = np.zeros((128, 128))
    jrev[np.arange(128), 127 - np.arange(128)] = 1.0
    small = np.concatenate([ld0, ld2, lda, ldb, rd0, rd2, rda, rdb, jrev], axis=0)
    return _pack_rows(small), _pack_rows(g.reshape(32, 128, 128))


def _dft4(z, inv):
    (ar, ai), (br, bi), (cr, ci), (dr, di) = z
    s0r, s0i = ar + cr, ai + ci
    s1r, s1i = ar - cr, ai - ci
    s2r, s2i = br + dr, bi + di
    s3r, s3i = br - dr, bi - di
    y0 = (s0r + s2r, s0i + s2i)
    y2 = (s0r - s2r, s0i - s2i)
    if not inv:
        y1 = (s1r + s3i, s1i - s3r)
        y3 = (s1r - s3i, s1i + s3r)
    else:
        y1 = (s1r - s3i, s1i + s3r)
        y3 = (s1r + s3i, s1i - s3r)
    return [y0, y1, y2, y3]


def _tw16(z, ex, inv):
    r, i = z
    ex = ex % 16
    if ex == 0:
        return z
    sgn = 1.0 if inv else -1.0
    if ex == 4:
        return (-i, r) if inv else (i, -r)
    c = float(np.cos(2 * np.pi * ex / 16))
    s = sgn * float(np.sin(2 * np.pi * ex / 16))
    if ex in (2, 6):
        h = float(np.sqrt(0.5))
        if c > 0 and s > 0:
            return ((r - i) * h, (r + i) * h)
        if c > 0 and s < 0:
            return ((r + i) * h, (i - r) * h)
        if c < 0 and s > 0:
            return ((r + i) * (-h), (r - i) * h)
        return ((i - r) * h, (r + i) * (-h))
    return (r * c - i * s, r * s + i * c)


def _dft16(z, inv):
    a = [None] * 16
    for n2 in range(4):
        y = _dft4([z[4 * n1 + n2] for n1 in range(4)], inv)
        for k1 in range(4):
            a[4 * k1 + n2] = _tw16(y[k1], k1 * n2, inv)
    out = [None] * 16
    for k1 in range(4):
        y = _dft4([a[4 * k1 + n2] for n2 in range(4)], inv)
        for k2 in range(4):
            out[k1 + 4 * k2] = y[k2]
    return out


def _unpack(w, idx):
    return pltpu.unpack_elementwise(w, index=idx, packed_dtype=BF16, unpacked_dtype=F32)


def _bf(w):
    return pltpu.bitcast(w, BF16)


def _u32(v):
    return pltpu.bitcast(v, U32)


def _kernel(one_hbm, x_hbm, wr_hbm, wi_hbm, w1_hbm, w2_hbm, gw_hbm, sm_hbm, g_hbm,
            o_hbm,
            xs, wrs, wis, nyq_r, nyq_i, w1s, w2s, gws, sm, gm,
            u_ref, t_ref, v_ref, a_ref, sp_ref, act, gate, os_, one_ref, sem):
    lane = lax.broadcasted_iota(jnp.int32, (1, 128), 1)
    lo_half = lane < 64
    even = (lane % 2) == 0
    cls_a = ((lane + 1) % 4) < 2
    row_even = (lax.broadcasted_iota(jnp.int32, (1, 8, 128), 1) % 2) == 0

    xb, w1b, w2b = xs.bitcast(BF16), w1s.bitcast(BF16), w2s.bitcast(BF16)
    wrb, wib = wrs.bitcast(BF16), wis.bitcast(BF16)
    vw, actw, ob = v_ref.bitcast(U32), act.bitcast(U32), os_

    def pk(lo, hi):
        return pltpu.pack_elementwise([lo, hi], packed_dtype=BF16).astype(U32)

    def group(k, pairs):
        return [pltpu.make_async_copy(s, d, sem.at[k]) for s, d in pairs]

    def start(cps):
        for c in cps:
            c.start()

    def wait(cps):
        for c in cps:
            c.wait()

    def w1_pairs(f0, f1):
        return [(w1_hbm.at[pl.ds(f0, f1 - f0), :], w1b.at[pl.ds(f0, f1 - f0), :])]

    def x_pairs(*blks):
        return [(x_hbm.at[pl.ds(256 * b, 256), :], xb.at[pl.ds(256 * b, 256), :]) for b in blks]

    d0 = group(0, w1_pairs(0, 128) + x_pairs(0) + [(one_hbm, one_ref)])
    d1 = group(1, w1_pairs(128, 256) + x_pairs(4))
    d2 = group(0, x_pairs(1) + w1_pairs(256, 512))
    d3 = group(1, x_pairs(5, 2, 6) + w1_pairs(512, 128 * NE))
    d4 = group(0, x_pairs(3, 7) + w1_pairs(128 * NE, 128 * NE + 128) + [(sm_hbm, sm), (gw_hbm, gws), (g_hbm, gm)])
    d5 = group(2, w1_pairs(128 * NE + 128, F)
               + [(wr_hbm.at[pl.ds(0, 256), :], wrb), (wi_hbm.at[pl.ds(0, 256), :], wib)]
               + [(wr_hbm.at[pl.ds(256, 1), :], nyq_r), (wi_hbm.at[pl.ds(256, 1), :], nyq_i)]
               + [(w2_hbm, w2b.at[pl.ds(0, F), :])])

    for d in (d0, d1):
        start(d)

    w2s[F // 2:FP // 2, :] = jnp.zeros(((FP - F) // 2, D), U32)
    t_ref[1, 0, 264:272, :] = jnp.zeros((8, 128), F32)
    a_ref[4 * AT:4 * AT + 8, :] = jnp.zeros((8, 128), F32)

    def after(w, zero):
        return jnp.concatenate([w[0:8] | pltpu.bitcast(zero, U32), w[8:]], axis=0)

    def after4(w, zeros):
        if zeros is None:
            return w
        return jnp.concatenate([after(w[16 * j:16 * j + 16], zeros[j]) for j in range(4)], axis=0)

    def mm1(ranges, nts):
        x = jnp.concatenate([_bf(xs[r0 // 2:r1 // 2, :]) for r0, r1 in ranges], axis=0)
        for nt in nts:
            w = _bf(w1s[64 * nt:64 * (nt + 1), :])
            h = lax.dot_general(x, w, NT, preferred_element_type=F32)
            hh = 0.5 * h
            th = jnp.tanh(hh)
            af = hh + hh * th
            a = af.astype(BF16)
            if nt == NF - 1:
                g = 0.5 * th[:, F - 1280:F - 1279] + 0.5
                gb = jnp.broadcast_to(g, (g.shape[0], 128))
            off = 0
            for r0, r1 in ranges:
                act[nt, r0:r1, :] = a[off:off + r1 - r0]
                if nt == NF - 1:
                    gate[r0:r1, :] = gb[off:off + r1 - r0]
                off += r1 - r0
        return af, a

    def f1(i, ps=range(8)):
        for p in ps:
            ew = 8 * i + p
            w = [[xs[512 * c + 16 * ew + 8 * o:512 * c + 16 * ew + 8 * o + 8, :] for c in range(2)]
                 for o in range(2)]
            for h in range(2):
                outs = []
                for o in range(2):
                    x0, x1 = _unpack(w[o][0], h), _unpack(w[o][1], h)
                    res = []
                    for zz in (x0 + x1, x0 - x1):
                        y0, y1, y2, y3 = [zz[:, 128 * t:128 * (t + 1)] for t in range(4)]
                        a0, a1 = y0 + y2, y1 + y3
                        pp, qq = y0 - y2, y1 - y3
                        ee = jnp.where(lo_half, pp, HQ * (pp + qq))
                        rr = pltpu.roll(jnp.where(lo_half, qq, HQ * (pp - qq)), 64, 1)
                        res.append((a0 + a1, a0 - a1, ee + rr, ee - rr))
                    outs.append(res)
                for kb in range(2):
                    for t in range(4):
                        u_ref[pl.ds(UB * h + 64 * t + 32 * kb + ew, 8, stride=2 * UB), :] = pk(
                            outs[0][kb][t], outs[1][kb][t])

    def phase_a1(s_lo, dep):
        u = [u_ref[UB * s_lo + 64 * t:UB * s_lo + 64 * t + 64, :] for t in range(4)]
        if dep is not None:
            u[0] = after(u[0], dep)
        u = [_bf(w) for w in u]
        o0 = lax.dot_general(_bf(sm[O_LD0:O_LD2, :]), u[0], NT, preferred_element_type=F32)
        o2 = lax.dot_general(_bf(sm[O_LD2:O_LDA, :]), u[1], NT, preferred_element_type=F32)
        oa = lax.dot_general(_bf(sm[O_LDA:O_LDB, :]), u[2], NT, preferred_element_type=F32)
        ob_ = lax.dot_general(_bf(sm[O_LDB:O_RD0, :]), u[3], NT, preferred_element_type=F32)
        r_e = pk(o0[0:64], o2[0:64])
        i_e = pk(o0[64:128], o2[64:128])
        oa, ob_ = oa.reshape(16, 8, 128), ob_.reshape(16, 8, 128)
        od = pk(jnp.where(row_even, oa, ob_).reshape(128, 128), jnp.where(row_even, ob_, oa).reshape(128, 128))
        r_o, i_o = od[0:64], od[64:128]
        r_n = pk(o0[128:136], o0[136:144])
        zero = jnp.zeros_like(r_n)
        r = jnp.concatenate([r_e, r_o], axis=0)
        t = pltpu.roll(jnp.concatenate([i_e, i_o], axis=0), 64, 1)
        la = _bf(jnp.concatenate([jnp.where(lo_half, r, t), jnp.where(lo_half, r_n, zero)], axis=0))
        lb = _bf(jnp.concatenate([jnp.where(lo_half, t, r), jnp.where(lo_half, zero, r_n)], axis=0))
        return la, lb

    def phase_a2(s_lo, la, lb):
        oa = jnp.dot(la, _bf(gm[2 * s_lo]), preferred_element_type=F32)[0:264]
        ob_ = jnp.dot(lb, _bf(gm[2 * s_lo + 1]), preferred_element_type=F32)[0:264]
        t_ref[s_lo, 0, 0:264, :] = jnp.where(even, oa, ob_)
        t_ref[s_lo, 1, 0:264, :] = pltpu.roll(jnp.where(even, ob_, oa), 127, 1)

    row8 = lax.broadcasted_iota(jnp.int32, (8, 128), 0)

    def special():
        row = lax.broadcasted_iota(jnp.int32, (16, S), 0)

        def rowcat(ref):
            return jnp.broadcast_to(
                _unpack(ref[0:1, :], 0), (16, S))
        q = jnp.where(row == 0, rowcat(wrs),
            jnp.where(row == 1, rowcat(wis),
            jnp.where(row == 2, jnp.broadcast_to(nyq_r[...].astype(F32), (16, S)),
            jnp.where(row == 3, jnp.broadcast_to(nyq_i[...].astype(F32), (16, S)), 0.0))))
        qb = q.astype(BF16)
        stacked = jnp.concatenate([qb[:, 128 * (15 - t):128 * (16 - t)] for t in range(16)], axis=0)
        rv = jnp.dot(stacked, _bf(sm[O_J:O_END, :]), preferred_element_type=F32)
        rev = jnp.concatenate([rv[16 * t:16 * t + 8] for t in range(16)], axis=1)
        mir = pltpu.roll(rev, 1, 1)
        sgn = jnp.where((lax.broadcasted_iota(jnp.int32, (8, S), 0) % 2) == 0, 1.0, -1.0)
        sp_ref[...] = q[0:8] + sgn * mir

    def ld(s, r0):
        return t_ref[s, 0, r0:r0 + 8, :], t_ref[s, 1, r0:r0 + 8, :]

    def st(s, r0, z):
        t_ref[s, 0, r0:r0 + 8, :] = z[0]
        t_ref[s, 1, r0:r0 + 8, :] = z[1]

    def sp_row(r, kt, other):
        return jnp.where(row8 == 0, jnp.broadcast_to(sp_ref[r:r + 1, 128 * kt:128 * (kt + 1)], (8, 128)), other)

    def p1(r0, n2):
        y = _dft4([ld(4 * n1 + n2, r0) for n1 in range(4)], False)
        for k1 in range(4):
            st(4 * k1 + n2, r0, _tw16(y[k1], k1 * n2, False))

    def p2(r0, k1):
        y = _dft4([ld(4 * k1 + n2, r0) for n2 in range(4)], False)
        u = []
        for k2 in range(4):
            kt = k1 + 4 * k2
            if r0 == 256:
                wr, wi = sp_row(2, kt, 0.0), sp_row(3, kt, 0.0)
            else:
                i8, h = r0 % 128, r0 // 128
                sl = slice(128 * kt, 128 * (kt + 1))
                wr, wi = _unpack(wrs[i8:i8 + 8, sl], h), _unpack(wis[i8:i8 + 8, sl], h)
                if r0 == 0:
                    wr, wi = sp_row(0, kt, wr), sp_row(1, kt, wi)
            xr, xi = y[k2]
            ur, ui = xr * wr - xi * wi, xr * wi + xi * wr
            if r0 == 0:
                er, ei = ld(4 * k1 + k2, 256)
                ur, ui = ur - ei, ui + er
            u.append((ur, ui))
        if r0 == 256:
            for k2 in range(4):
                st(4 * k1 + k2, r0, u[k2])
            return
        y = _dft4(u, True)
        for n2 in range(4):
            st(4 * k1 + n2, r0, _tw16(y[n2], k1 * n2, True))

    def p3(r0, n2):
        y = _dft4([ld(4 * k1 + n2, r0) for k1 in range(4)], True)
        for n1 in range(4):
            v_ref[4 * n1 + n2, 0, r0:r0 + 8, :] = y[n1][0].astype(BF16)
            v_ref[4 * n1 + n2, 1, r0:r0 + 8, :] = y[n1][1].astype(BF16)

    def phase_c1(s_lo, dep):
        vr = vw[s_lo, 0]
        t = pltpu.roll(vw[s_lo, 1], 1, 1)
        va = _bf(jnp.where(even, vr, t))
        vb = _bf(jnp.where(even, t, vr))
        za = lax.dot_general(_bf(after4(gm[2 * s_lo], dep)), va, NT, preferred_element_type=F32)
        zb = lax.dot_general(_bf(gm[2 * s_lo + 1]), vb, NT, preferred_element_type=F32)
        zr = pk(za[0:64] + zb[64:128], za[0:64] - zb[64:128])
        zi = pk(za[64:128] + zb[0:64], za[64:128] - zb[0:64])
        re = zr[:, 0:128]
        t = pltpu.roll(zi[:, 0:128], 1, 1)
        l0 = jnp.where(even, re, t)
        l2 = _bf(jnp.where(even, t, re))
        ro = zr[:, 128:256]
        t = pltpu.roll(zi[:, 128:256], 2, 1)
        la = _bf(jnp.where(cls_a, ro, t))
        lb = _bf(jnp.where(cls_a, t, ro))
        return l0, l2, la, lb

    def phase_c2(s_lo, dep, want, l0, l2, la, lb):
        a0 = jnp.dot(_bf(after4(l0, dep)), _bf(sm[O_RD0:O_RD2, :]), preferred_element_type=F32)
        a2 = jnp.dot(l2, _bf(sm[O_RD2:O_RDA, :]), preferred_element_type=F32)
        va = jnp.dot(la, _bf(sm[O_RDA:O_RDB, :]), preferred_element_type=F32)
        vb = jnp.dot(lb, _bf(sm[O_RDB:O_J, :]), preferred_element_type=F32)
        ee = va + vb
        cc = pltpu.roll(va - vb, 64, 1)
        pp = jnp.where(lo_half, ee, HQ * (ee + cc))
        qq = jnp.where(lo_half, cc, HQ * (ee - cc))
        e0, e1 = a0 + a2, a0 - a2
        ys = [e0 + pp, e1 + qq, e0 - pp, e1 - qq]
        zeros = []
        for k in range(8):
            for t, y in enumerate(ys):
                a_ref[pl.ds(AT * t + s_lo + 16 * k * AS, 16, stride=AS), :] = y[16 * k:16 * k + 16]
            if want:
                zeros.append(a_ref[pl.ds(4 * AT + z, 8), :])
        return zeros

    def mm2(r0, r1, split):
        lhs = jnp.concatenate([_bf(actw[nt, r0 // 2:r1 // 2, :]) for nt in range(NF)], axis=1)
        w2 = _bf(w2s[...])
        b = jnp.dot(lhs, w2, preferred_element_type=F32)
        g = gate[r0:r1, :]
        cps = []
        for t in range(4):
            bt = b[:, 128 * t:128 * (t + 1)]
            pos = [AT * t + AS * (2 * ((r % 1024) // 16) + r // 1024) for r in range(r0, r1, 16)]
            at = jnp.concatenate([a_ref[p:p + 16, :] for p in pos], axis=0)
            ob[r0:r1, 128 * t:128 * (t + 1)] = (bt + g * (at - bt)).astype(BF16)
            if split:
                cp = group(0, [(ob.at[pl.ds(r0, r1 - r0), pl.ds(128 * t, 128)],
                                o_hbm.at[pl.ds(r0, r1 - r0), pl.ds(128 * t, 128)])])
                start(cp)
                cps += cp
        if not split:
            cps = group(0, [(ob.at[pl.ds(r0, r1 - r0), :], o_hbm.at[pl.ds(r0, r1 - r0), :])])
            start(cps)
        return cps

    def tok(v):
        t_ref[0, 0, pl.ds(264 + z, 8), :] = v

    def tok_u(v):
        u_ref[pl.ds(16 * UB + z, 8), :] = pltpu.bitcast(v, U32)

    def blk(*bs):
        return [(256 * b, 256 * b + 256) for b in bs]

    def mm1_f1(units, f1s):
        res = [mm1(blk(*bs), (nt,))[0] for bs, nt in units]
        rows = [(k, r) for k, a in enumerate(res) for r in range(0, a.shape[0], 16)]
        step = max(len(rows) - 8, 1) / max(len(f1s), 1)
        for j, (i, p) in enumerate(f1s):
            k, r = rows[int(j * step)]
            tok_u(res[k][r:r + 8])
            f1(i, (p,))

    wait(d0)
    start(d2)
    z = one_ref[0] - 1
    mm1(blk(0), (0,))
    wait(d1)
    start(d3)
    mm1_f1([((0,), 1), ((4,), 0), ((4,), 1)], [(0, p) for p in range(4)])
    wait(d2)
    start(d4)
    start(d5)
    mm1_f1([((1,), 0), ((1,), 1)] + [((0, 4, 1), nt) for nt in range(2, 4)], [(0, p) for p in range(4, 8)])
    wait(d3)
    mm1_f1([((5, 2, 6), nt) for nt in range(NE)] + [((0, 4, 1), nt) for nt in range(4, NE)],
           [(i, p) for i in (1, 2) for p in range(8)])
    wait(d4)
    gw = gws[...].reshape(1, D).astype(F32)
    rowp = lax.broadcasted_iota(jnp.int32, (FP - F, D), 0)
    padv = _u32(jnp.where(rowp == 0, jnp.broadcast_to(gw, (FP - F, D)), 0.0).astype(BF16))
    w1s[F // 2:FP // 2, :] = padv
    mm1_f1([((3, 7), nt) for nt in range(NE - 3)], [(3, p) for p in range(8)])
    mm1(blk(3, 7), (NE - 3,))

    pend = []
    deps = {}
    for s_lo in range(16 + LAG):
        if s_lo < 16:
            pend.append(phase_a1(s_lo, deps.get(s_lo)))
        if 2 <= s_lo and s_lo + DA < 16:
            deps[s_lo + DA] = t_ref[1, 0, pl.ds(264 + z, 8), :]
        if s_lo == 16:
            mm1(blk(3, 7), (NE - 2,))
        if s_lo >= LAG:
            phase_a2(s_lo - LAG, *pend[s_lo - LAG])
    mm1(blk(3, 7), (NE - 1,))
    mm1([(0, 512)], (NE,))

    wait(d5)
    rgs = [8 * i for i in range(1, 32)] + [256, 0]
    slots = []
    for j in range(len(rgs) + 2):
        for a in range(4):
            job = []
            if j < len(rgs):
                job.append((p1, rgs[j], a))
            if 0 <= j - 2 < len(rgs) and rgs[j - 2] != 256:
                job.append((p3, rgs[j - 2], a))
            if job:
                slots.append(job)
            if 0 <= j - 1 < len(rgs):
                slots.append([(p2, rgs[j - 1], a)])
    units = [(q, nt) for nt in range(NE, NF) for q in range(4)][1:]
    total = len(units) * 512
    step = (total - 320) / len(slots)
    j = 0
    for k, (q, nt) in enumerate(units):
        af = mm1([(512 * q, 512 * q + 512)], (nt,))[0]
        if k == 2:
            special()
        while j < len(slots) and int(j * step) < 512 * (k + 1):
            r = ((int(j * step) - 512 * k) // 8) * 8
            tok(af[r:r + 8])
            for fn, r0, a in slots[j]:
                fn(r0, a)
            j += 1

    pend = []
    zs = {}
    for s_lo in range(17):
        if s_lo < 16:
            pend.append(phase_c1(s_lo, zs[s_lo - DC - 1][0:4] if s_lo - DC - 1 >= 0 else None))
        if s_lo >= 1:
            sg = s_lo - 1
            zs[sg] = phase_c2(sg, zs[sg - DC][4:8] if sg - DC >= 0 else None, sg + DC < 16, *pend[sg])

    outs = []
    for r0, r1 in [(0, 512), (512, 1024), (1024, 1536), (1536, 1920), (1920, 2048)]:
        outs += mm2(r0, r1, r1 == S)
    wait(outs)


@jax.jit
def pallas_gated_mix__spectral_gfnet__dense_activation_silu__prompt_kernel(A_x, A_w_r, A_w_i, B_x, B_w1, B_w2, gate_w):
    small, g = _consts()
    out = pl.pallas_call(
        _kernel,
        out_shape=jax.ShapeDtypeStruct((S, D), BF16),
        in_specs=[pl.BlockSpec(memory_space=pl.ANY)] * 9,
        out_specs=pl.BlockSpec(memory_space=pl.ANY),
        scratch_shapes=[
            pltpu.VMEM((S // 2, D), U32),
            pltpu.VMEM((128, S), U32),
            pltpu.VMEM((128, S), U32),
            pltpu.VMEM((1, S), BF16),
            pltpu.VMEM((1, S), BF16),
            pltpu.VMEM((FP // 2, D), U32),
            pltpu.VMEM((FP // 2, D), U32),
            pltpu.VMEM((D,), BF16),
            pltpu.VMEM((O_END, 128), U32),
            pltpu.VMEM((32, 64, 128), U32),
            pltpu.VMEM((18 * UB, 128), U32),
            pltpu.VMEM((16, 2, 272, 128), F32),
            pltpu.VMEM((16, 2, 256, 128), BF16),
            pltpu.VMEM((4 * AT + 32, 128), F32),
            pltpu.VMEM((8, S), F32),
            pltpu.VMEM((NF, S, 128), BF16),
            pltpu.VMEM((S, 128), F32),
            pltpu.VMEM((S, D), BF16),
            pltpu.SMEM((128,), jnp.int32),
            pltpu.SemaphoreType.DMA((3,)),
        ],
        compiler_params=pltpu.CompilerParams(vmem_limit_bytes=100 * 1024 * 1024),
    )(jnp.asarray(np.arange(1, 129, dtype=np.int32)), A_x[0], A_w_r.T, A_w_i.T, B_w1.T, B_w2, gate_w, jnp.asarray(small), jnp.asarray(g))
    return out[None]
```

```python
import numpy as np
import jax
import jax.numpy as jnp
from jax import lax
import jax.experimental.pallas as pl
import jax.experimental.pallas.tpu as pltpu

S, D, F = 2048, 512, 1376
FP = 1408
NF = 11
NT = (((1,), (1,)), ((), ()))
AS = 20
AT = AS * 128
UB = 258
WS_END = 704 + 960
MM2_CHUNKS = [(0, 256), (256, 512), (512, 768), (768, 896), (896, 1024)]
LAG, DA, DC, TOKC = 1, 3, 2, 15
SW, NSB, BT, F1S, F1T = 0.8, 4, 1200, 4, 5
HQ = float(np.sqrt(0.5))
F32 = jnp.float32
BF16 = jnp.bfloat16
U32 = jnp.uint32

O_LD0, O_LD2, O_LDA, O_LDB, O_RD0, O_RD2, O_RDA, O_RDB, O_J, O_END = 0, 72, 136, 200, 264, 328, 392, 456, 520, 584


def _pack_rows(a):
    f = np.ascontiguousarray(a, dtype=np.float32)
    u = f.view(np.uint32).astype(np.uint64)
    b = ((u + 0x7FFF + ((u >> 16) & 1)) >> 16).astype(np.uint32)
    return (b[..., 0::2, :] | (b[..., 1::2, :] << 16)).astype(np.uint32)


def _consts():
    n2 = np.arange(128)
    j = np.arange(64)
    ld0 = np.zeros((144, 128))
    th = 2 * np.pi * np.outer(4 * j, n2) / 512
    ld0[0:64] = np.cos(th)
    ld0[64:128] = -np.sin(th)
    ld0[128] = np.cos(np.pi * n2)
    ld2 = np.zeros((128, 128))
    th = 2 * np.pi * np.outer(4 * j + 2, n2) / 512
    ld2[0:64] = np.cos(th)
    ld2[64:128] = -np.sin(th)
    i = np.arange(128)
    th = 2 * np.pi * np.outer(2 * i + 1, n2) / 512
    sg = np.where(i % 2 == 0, -1.0, 1.0)[:, None]
    ld1 = np.zeros((256, 256))
    ld1[0:128, 0:128] = np.cos(th)
    ld1[0:128, 128:256] = sg * np.sin(th)
    ld1[128:256, 0:128] = -np.sin(th)
    ld1[128:256, 128:256] = sg * np.cos(th)
    sc = 2.0 / (S * D)
    rd0 = np.zeros((128, 128))
    rd0[0::2] = ld0[0:64] * sc
    rd0[1::2] = ld0[64:128] * sc
    rd0[0] = ld0[0] * sc / 4
    rd0[1] = ld0[128] * sc / 4
    rd2 = np.zeros((128, 128))
    rd2[1::2] = ld2[0:64] * sc
    rd2[(2 * j + 2) % 128] = ld2[64:128] * sc
    hq = np.sqrt(0.5)
    eye, n64 = np.eye(256), np.arange(64)
    p_, q_ = eye[:, 0:128], eye[:, 128:256]
    lo = (np.arange(128) < 64)[None, :]
    e_ = np.where(lo, p_, hq * (p_ + q_))
    c_ = np.where(lo, q_, hq * (p_ - q_))
    r_ = np.roll(c_, 64, axis=1)
    mm = np.concatenate([e_ + r_, e_ - r_], axis=1).T
    ldv = ld1 @ mm.T / 2
    cls_a = (i % 4 == 0) | (i % 4 == 3)
    assert np.abs(ldv[np.concatenate([cls_a, cls_a])][:, 128:]).max() < 1e-9
    assert np.abs(ldv[np.concatenate([~cls_a, ~cls_a])][:, :128]).max() < 1e-9
    sg_ = np.arange(64)
    ia = np.where(sg_ % 2 == 0, 2 * sg_, 2 * sg_ + 1)
    ib = np.where(sg_ % 2 == 0, 2 * sg_ + 1, 2 * sg_)
    lda = np.concatenate([ldv[ia, :128], ldv[128 + ia, :128]], axis=0)
    ldb = np.concatenate([ldv[ib, 128:], ldv[128 + ib, 128:]], axis=0)
    rda, rdb = np.zeros((128, 128)), np.zeros((128, 128))
    ia_, ib_ = i[cls_a], i[~cls_a]
    rda[ia_] = ldv[ia_, :128] * sc
    rda[(ia_ + 2) % 128] = ldv[128 + ia_, :128] * sc
    rdb[ib_] = ldv[ib_, 128:] * sc
    rdb[(ib_ + 2) % 128] = ldv[128 + ib_, 128:] * sc
    e = np.arange(64)
    kl = np.arange(64)
    g = np.zeros((16, 2, 128, 128))
    for s_lo in range(16):
        for kb in range(2):
            th = -2 * np.pi * np.outer(s_lo + 16 * e, 2 * kl + kb) / S
            gr, gi = np.cos(th), np.sin(th)
            if kb == 0:
                rr, ri = slice(0, 64), slice(64, 128)
                cr, ci = 2 * kl, 2 * kl + 1
            else:
                rr, ri = slice(64, 128), slice(0, 64)
                cr, ci = 2 * kl + 1, (2 * kl + 2) % 128
            m = np.zeros((128, 128))
            m[rr, cr] = gr
            m[rr, ci] = gi
            m[ri, cr] = -gi
            m[ri, ci] = gr
            g[s_lo, kb] = m
    jrev = np.zeros((128, 128))
    jrev[np.arange(128), 127 - np.arange(128)] = 1.0
    small = np.concatenate([ld0, ld2, lda, ldb, rd0, rd2, rda, rdb, jrev], axis=0)
    return _pack_rows(small), _pack_rows(g.reshape(32, 128, 128))


def _dft4(z, inv):
    (ar, ai), (br, bi), (cr, ci), (dr, di) = z
    s0r, s0i = ar + cr, ai + ci
    s1r, s1i = ar - cr, ai - ci
    s2r, s2i = br + dr, bi + di
    s3r, s3i = br - dr, bi - di
    y0 = (s0r + s2r, s0i + s2i)
    y2 = (s0r - s2r, s0i - s2i)
    if not inv:
        y1 = (s1r + s3i, s1i - s3r)
        y3 = (s1r - s3i, s1i + s3r)
    else:
        y1 = (s1r - s3i, s1i + s3r)
        y3 = (s1r + s3i, s1i - s3r)
    return [y0, y1, y2, y3]


def _tw16(z, ex, inv):
    r, i = z
    ex = ex % 16
    if ex == 0:
        return z
    sgn = 1.0 if inv else -1.0
    if ex == 4:
        return (-i, r) if inv else (i, -r)
    c = float(np.cos(2 * np.pi * ex / 16))
    s = sgn * float(np.sin(2 * np.pi * ex / 16))
    if ex in (2, 6):
        h = float(np.sqrt(0.5))
        if c > 0 and s > 0:
            return ((r - i) * h, (r + i) * h)
        if c > 0 and s < 0:
            return ((r + i) * h, (i - r) * h)
        if c < 0 and s > 0:
            return ((r + i) * (-h), (r - i) * h)
        return ((i - r) * h, (r + i) * (-h))
    return (r * c - i * s, r * s + i * c)


def _dft16(z, inv):
    a = [None] * 16
    for n2 in range(4):
        y = _dft4([z[4 * n1 + n2] for n1 in range(4)], inv)
        for k1 in range(4):
            a[4 * k1 + n2] = _tw16(y[k1], k1 * n2, inv)
    out = [None] * 16
    for k1 in range(4):
        y = _dft4([a[4 * k1 + n2] for n2 in range(4)], inv)
        for k2 in range(4):
            out[k1 + 4 * k2] = y[k2]
    return out


def _unpack(w, idx):
    bits = (w << 16) if idx == 0 else (w & jnp.uint32(0xFFFF0000))
    return lax.bitcast_convert_type(bits, F32)


def _bf(w):
    return pltpu.bitcast(w, BF16)


def _u32(v):
    return pltpu.bitcast(v, U32)


def _kernel(one_hbm, x_hbm, wr_hbm, wi_hbm, w1_hbm, w2_hbm, gw_hbm, sm_hbm, g_hbm,
            o_hbm,
            xs, wrs, wis, nyq_r, nyq_i, dc_r, dc_i, w1s, w2s, gws, sm, gm,
            u_ref, t_a, t_b, v_ref, a_ref, sp_ref, act, gate, os_, xs0, xs1, xs2, xs3, wq0, wq1, wq2, wq3, wq4, one_ref, sem):
    xsum, wsum = (xs0, xs1, xs2, xs3), (wq0, wq1, wq2, wq3, wq4)
    xsumw = [r.bitcast(U32) for r in xsum]
    wsumw = [r.bitcast(U32) for r in wsum]
    lane = lax.broadcasted_iota(jnp.int32, (1, 128), 1)
    lo_half = lane < 64
    even = (lane % 2) == 0
    cls_a = ((lane + 1) % 4) < 2
    row_even = (lax.broadcasted_iota(jnp.int32, (1, 8, 128), 1) % 2) == 0

    xb, w1b, w2b = xs.bitcast(BF16), w1s.bitcast(BF16), w2s.bitcast(BF16)
    wrb, wib = wrs.bitcast(BF16), wis.bitcast(BF16)
    vw, actw, ob = v_ref.bitcast(U32), act.bitcast(U32), os_

    def pk(lo, hi):
        half = jnp.uint32(0x8000)
        lo = (lax.bitcast_convert_type(lo, U32) + half) >> 16
        hi = (lax.bitcast_convert_type(hi, U32) + half) & jnp.uint32(0xFFFF0000)
        return lo | hi

    def group(k, pairs):
        return [pltpu.make_async_copy(s, d, sem.at[k]) for s, d in pairs]

    def start(cps):
        for c in cps:
            c.start()

    def wait(cps):
        for c in cps:
            c.wait()

    def w1_pairs(f0, f1):
        return [(w1_hbm.at[pl.ds(f0, f1 - f0), :], w1b.at[pl.ds(f0, f1 - f0), :])]

    def x_pairs(*blks):
        return [(x_hbm.at[pl.ds(256 * b, 256), :], xb.at[pl.ds(256 * b, 256), :]) for b in blks]

    d0 = group(0, w1_pairs(0, 128) + x_pairs(0) + [(one_hbm, one_ref)])
    d1 = group(1, w1_pairs(128, 256) + x_pairs(4))
    d2 = group(0, x_pairs(1) + w1_pairs(256, 512))
    d3 = group(1, x_pairs(5, 2, 6) + w1_pairs(512, 768))
    d4 = group(0, x_pairs(3, 7) + [(sm_hbm, sm), (gw_hbm, gws), (g_hbm, gm)]
               + [(wr_hbm.at[pl.ds(256, 1), :], nyq_r), (wi_hbm.at[pl.ds(256, 1), :], nyq_i)]
               + [(wr_hbm.at[pl.ds(0, 16), :], dc_r), (wi_hbm.at[pl.ds(0, 16), :], dc_i)])
    d5 = group(2, w1_pairs(768, F)
               + [(wr_hbm.at[pl.ds(0, 256), :], wrb), (wi_hbm.at[pl.ds(0, 256), :], wib)]
               + [(w2_hbm, w2b.at[pl.ds(0, F), :])])

    for d in (d0, d1):
        start(d)

    w2s[F // 2:FP // 2, :] = jnp.zeros(((FP - F) // 2, D), U32)
    t_a[1, 0, 136:144, :] = jnp.zeros((8, 128), F32)
    t_b[1, 0, 136:144, :] = jnp.zeros((8, 128), F32)

    def tloc(r0):
        return (t_b, r0 - 128) if 128 <= r0 < 256 else (t_a, min(r0, 128))
    a_ref[4 * AT:4 * AT + 8, :] = jnp.zeros((8, 128), F32)

    def after(w, zero):
        return jnp.concatenate([w[0:8] | pltpu.bitcast(zero, U32), w[8:]], axis=0)

    def after4(w, zeros):
        if zeros is None:
            return w
        return jnp.concatenate([after(w[16 * j:16 * j + 16], zeros[j]) for j in range(4)], axis=0)

    def addbf(p, q, sign):
        p, q = p.astype(F32), q.astype(F32)
        return (p + q if sign > 0 else p - q).astype(BF16)

    def silu_store(h, ranges, nt):
        hh = 0.5 * h
        th = jnp.tanh(hh)
        a = (hh + hh * th).astype(BF16)
        if nt == NF - 1:
            g = 0.5 * th[:, F - 1280:F - 1279] + 0.5
            gb = jnp.broadcast_to(g, (g.shape[0], 128))
        off = 0
        for r0, r1 in ranges:
            act[nt, r0:r1, :] = a[off:off + r1 - r0]
            if nt == NF - 1:
                gate[r0:r1, :] = gb[off:off + r1 - r0]
            off += r1 - r0

    def ntdot(a, b):
        return lax.dot_general(a, b, NT, preferred_element_type=F32)

    def mm1(bs, nt):
        ranges = [(256 * b, 256 * b + 256) for b in bs]
        x = jnp.concatenate([_bf(xs[r0 // 2:r1 // 2, :]) for r0, r1 in ranges], axis=0)
        h = ntdot(x, _bf(w1s[64 * nt:64 * (nt + 1), :]))
        silu_store(h, ranges, nt)
        return 256 * len(bs), lambda t: h[(t // 8) * 8:(t // 8) * 8 + 8]

    def x_mini(p, i, n):
        for t in range(2):
            a11, a12, a21, a22 = [
                _bf(xs[512 * mh + 128 * p + 8 * i:512 * mh + 128 * p + 8 * (i + n),
                       256 * kh + 128 * t:256 * kh + 128 * t + 128]).astype(F32)
                for mh in range(2) for kh in range(2)]
            for k, v in enumerate([a11 + a22, a21 + a22, a11 + a12, a21 - a11, a12 - a22]):
                xsum[p][2 * k + t, 16 * i:16 * (i + n), :] = v.astype(BF16)

    def w1_mini(tp, i, n):
        for t in range(2):
            b11, b12, b21, b22 = [
                _bf(w1s[128 * tp + 64 * nh + 8 * i:128 * tp + 64 * nh + 8 * (i + n),
                        256 * kh + 128 * t:256 * kh + 128 * t + 128]).astype(F32)
                for kh in range(2) for nh in range(2)]
            for k, v in enumerate([b11 + b22, b12 - b22, b21 - b11, b11 + b12, b21 + b22]):
                wsum[tp][2 * k + t, 16 * i:16 * (i + n), :] = v.astype(BF16)

    def mm1s(p, tp):
        a11 = _bf(xs[128 * p:128 * p + 128, 0:256])
        a22 = _bf(xs[512 + 128 * p:512 + 128 * p + 128, 256:512])
        b11 = _bf(w1s[128 * tp:128 * tp + 64, 0:256])
        b22 = _bf(w1s[128 * tp + 64:128 * tp + 128, 256:512])
        sa = [jnp.concatenate([_bf(xsumw[p][2 * k]), _bf(xsumw[p][2 * k + 1])], axis=1) for k in range(5)]
        sb = [jnp.concatenate([_bf(wsumw[tp][2 * k]), _bf(wsumw[tp][2 * k + 1])], axis=1) for k in range(5)]
        top, bot = [(256 * p, 256 * p + 256)], [(1024 + 256 * p, 1024 + 256 * p + 256)]
        m3 = ntdot(a11, sb[1])
        m5 = ntdot(sa[2], b22)
        silu_store(m3 + m5, top, 2 * tp + 1)
        m4 = ntdot(a22, sb[2])
        m2 = ntdot(sa[1], b11)
        silu_store(m2 + m4, bot, 2 * tp)
        m1 = ntdot(sa[0], sb[0])
        m7 = ntdot(sa[4], sb[4])
        silu_store((m4 - m5) + m1 + m7, top, 2 * tp)
        m6 = jnp.concatenate([ntdot(sa[3][0:128], sb[3]), ntdot(sa[3][128:256], sb[3])], axis=0)
        silu_store((m3 - m2 + m1) + m6, bot, 2 * tp + 1)
        ms = (m3, m4, m1, m6)
        return 896, lambda t: ms[t // 256][((t % 256) // 8) * 8:((t % 256) // 8) * 8 + 8]

    def f1(i, ps=range(8)):
        for p in ps:
            ew = 8 * i + p
            w = [[xs[512 * c + 16 * ew + 8 * o:512 * c + 16 * ew + 8 * o + 8, :] for c in range(2)]
                 for o in range(2)]
            for h in range(2):
                outs = []
                for o in range(2):
                    x0, x1 = _unpack(w[o][0], h), _unpack(w[o][1], h)
                    res = []
                    for zz in (x0 + x1, x0 - x1):
                        y0, y1, y2, y3 = [zz[:, 128 * t:128 * (t + 1)] for t in range(4)]
                        a0, a1 = y0 + y2, y1 + y3
                        pp, qq = y0 - y2, y1 - y3
                        ee = jnp.where(lo_half, pp, HQ * (pp + qq))
                        rr = pltpu.roll(jnp.where(lo_half, qq, HQ * (pp - qq)), 64, 1)
                        res.append((a0 + a1, a0 - a1, ee + rr, ee - rr))
                    outs.append(res)
                for kb in range(2):
                    for t in range(4):
                        u_ref[pl.ds(UB * h + 64 * t + 32 * kb + ew, 8, stride=2 * UB), :] = pk(
                            outs[0][kb][t], outs[1][kb][t])

    def phase_a1(s_lo, dep):
        u = [u_ref[UB * s_lo + 64 * t:UB * s_lo + 64 * t + 64, :] for t in range(4)]
        if dep is not None:
            u[0] = after(u[0], dep)
        u = [_bf(w) for w in u]
        o0 = lax.dot_general(_bf(sm[O_LD0:O_LD2, :]), u[0], NT, preferred_element_type=F32)
        o2 = lax.dot_general(_bf(sm[O_LD2:O_LDA, :]), u[1], NT, preferred_element_type=F32)
        oa = lax.dot_general(_bf(sm[O_LDA:O_LDB, :]), u[2], NT, preferred_element_type=F32)
        ob_ = lax.dot_general(_bf(sm[O_LDB:O_RD0, :]), u[3], NT, preferred_element_type=F32)
        r_e = pk(o0[0:64], o2[0:64])
        i_e = pk(o0[64:128], o2[64:128])
        oa, ob_ = oa.reshape(16, 8, 128), ob_.reshape(16, 8, 128)
        od = pk(jnp.where(row_even, oa, ob_).reshape(128, 128), jnp.where(row_even, ob_, oa).reshape(128, 128))
        r_o, i_o = od[0:64], od[64:128]
        r_n = pk(o0[128:136], o0[136:144])
        zero = jnp.zeros_like(r_n)
        r = jnp.concatenate([r_e, r_o], axis=0)
        t = pltpu.roll(jnp.concatenate([i_e, i_o], axis=0), 64, 1)
        la = _bf(jnp.concatenate([jnp.where(lo_half, r, t), jnp.where(lo_half, r_n, zero)], axis=0))
        lb = _bf(jnp.concatenate([jnp.where(lo_half, t, r), jnp.where(lo_half, zero, r_n)], axis=0))
        return la, lb

    def phase_a2(s_lo, la, lb):
        oa = jnp.dot(la, _bf(gm[2 * s_lo]), preferred_element_type=F32)[0:264]
        ob_ = jnp.dot(lb, _bf(gm[2 * s_lo + 1]), preferred_element_type=F32)[0:264]
        for ri, v in enumerate((jnp.where(even, oa, ob_), pltpu.roll(jnp.where(even, ob_, oa), 127, 1))):
            t_a[s_lo, ri, 0:128, :] = v[0:128]
            t_b[s_lo, ri, 0:128, :] = v[128:256]
            t_a[s_lo, ri, 128:136, :] = v[256:264]

    row8 = lax.broadcasted_iota(jnp.int32, (8, 128), 0)

    def special():
        row = lax.broadcasted_iota(jnp.int32, (16, S), 0)

        def rowcat(ref):
            return jnp.broadcast_to(
                ref[0:1, :].astype(F32), (16, S))
        q = jnp.where(row == 0, rowcat(dc_r),
            jnp.where(row == 1, rowcat(dc_i),
            jnp.where(row == 2, jnp.broadcast_to(nyq_r[...].astype(F32), (16, S)),
            jnp.where(row == 3, jnp.broadcast_to(nyq_i[...].astype(F32), (16, S)), 0.0))))
        qb = q.astype(BF16)
        stacked = jnp.concatenate([qb[:, 128 * (15 - t):128 * (16 - t)] for t in range(16)], axis=0)
        rv = jnp.dot(stacked, _bf(sm[O_J:O_END, :]), preferred_element_type=F32)
        rev = jnp.concatenate([rv[16 * t:16 * t + 8] for t in range(16)], axis=1)
        mir = pltpu.roll(rev, 1, 1)
        sgn = jnp.where((lax.broadcasted_iota(jnp.int32, (8, S), 0) % 2) == 0, 1.0, -1.0)
        sp_ref[...] = q[0:8] + sgn * mir

    def ld(s, r0, n=8):
        ref, r = tloc(r0)
        return ref[s, 0, r:r + n, :], ref[s, 1, r:r + n, :]

    def st(s, r0, z):
        ref, r = tloc(r0)
        ref[s, 0, r:r + 8, :] = z[0]
        ref[s, 1, r:r + 8, :] = z[1]

    def sp_row(r, kt, other):
        return jnp.where(row8 == 0, jnp.broadcast_to(sp_ref[r:r + 1, 128 * kt:128 * (kt + 1)], (8, 128)), other)

    def p1(r0, n2):
        y = _dft4([ld(4 * n1 + n2, r0) for n1 in range(4)], False)
        for k1 in range(4):
            st(4 * k1 + n2, r0, _tw16(y[k1], k1 * n2, False))

    def p2(r0, k1):
        y = _dft4([ld(4 * k1 + n2, r0) for n2 in range(4)], False)
        u = []
        for k2 in range(4):
            kt = k1 + 4 * k2
            if r0 == 256:
                wr, wi = sp_row(2, kt, 0.0), sp_row(3, kt, 0.0)
            else:
                i8, h = r0 % 128, r0 // 128
                sl = slice(128 * kt, 128 * (kt + 1))
                rows = pl.ds(i8, 8) if h == 0 else pl.ds(pl.multiple_of(i8 + 8 * z, 8), 8)
                wr, wi = _unpack(wrs[rows, sl], h), _unpack(wis[rows, sl], h)
                if r0 == 0:
                    wr, wi = sp_row(0, kt, wr), sp_row(1, kt, wi)
            xr, xi = y[k2]
            ur, ui = xr * wr - xi * wi, xr * wi + xi * wr
            if r0 == 0:
                er, ei = ld(4 * k1 + k2, 256)
                ur, ui = ur - ei, ui + er
            u.append((ur, ui))
        if r0 == 256:
            for k2 in range(4):
                st(4 * k1 + k2, r0, u[k2])
            return
        y = _dft4(u, True)
        for n2 in range(4):
            st(4 * k1 + n2, r0, _tw16(y[n2], k1 * n2, True))

    def p3(r0, n2):
        y = _dft4([ld(4 * k1 + n2, r0, 16) for k1 in range(4)], True)
        for n1 in range(4):
            v_ref[4 * n1 + n2, 0, r0:r0 + 16, :] = y[n1][0].astype(BF16)
            v_ref[4 * n1 + n2, 1, r0:r0 + 16, :] = y[n1][1].astype(BF16)

    def phase_c1(s_lo, dep):
        vr = vw[s_lo + z, 0]
        t = pltpu.roll(vw[s_lo + z, 1], 1, 1)
        va = _bf(jnp.where(even, vr, t))
        vb = _bf(jnp.where(even, t, vr))
        za = lax.dot_general(_bf(after4(gm[2 * s_lo], dep)), va, NT, preferred_element_type=F32)
        zb = lax.dot_general(_bf(gm[2 * s_lo + 1]), vb, NT, preferred_element_type=F32)
        zr = pk(za[0:64] + zb[64:128], za[0:64] - zb[64:128])
        zi = pk(za[64:128] + zb[0:64], za[64:128] - zb[0:64])
        re = zr[:, 0:128]
        t = pltpu.roll(zi[:, 0:128], 1, 1)
        l0 = jnp.where(even, re, t)
        l2 = _bf(jnp.where(even, t, re))
        ro = zr[:, 128:256]
        t = pltpu.roll(zi[:, 128:256], 2, 1)
        la = _bf(jnp.where(cls_a, ro, t))
        lb = _bf(jnp.where(cls_a, t, ro))
        return l0, l2, la, lb

    def phase_c2(s_lo, dep, want, l0, l2, la, lb):
        a0 = jnp.dot(_bf(after4(l0, dep)), _bf(sm[O_RD0:O_RD2, :]), preferred_element_type=F32)
        a2 = jnp.dot(l2, _bf(sm[O_RD2:O_RDA, :]), preferred_element_type=F32)
        va = jnp.dot(la, _bf(sm[O_RDA:O_RDB, :]), preferred_element_type=F32)
        vb = jnp.dot(lb, _bf(sm[O_RDB:O_J, :]), preferred_element_type=F32)
        ee = va + vb
        cc = pltpu.roll(va - vb, 64, 1)
        pp = jnp.where(lo_half, ee, HQ * (ee + cc))
        qq = jnp.where(lo_half, cc, HQ * (ee - cc))
        e0, e1 = a0 + a2, a0 - a2
        ys = [e0 + pp, e1 + qq, e0 - pp, e1 - qq]
        zeros = []
        for k in range(8):
            for t, y in enumerate(ys):
                a_ref[pl.ds(AT * t + s_lo + 16 * k * AS, 16, stride=AS), :] = y[16 * k:16 * k + 16]
            if want:
                zeros.append(a_ref[pl.ds(4 * AT + z, 8), :])
        return zeros

    def ws_pos(k):
        return FP + 640 * (k // 2), 256 * (k % 2)

    def w2_mini(i, n):
        for t in range(2):
            b11, b12, b21, b22 = [
                _bf(w2s[320 * kh + 8 * i:320 * kh + 8 * (i + n),
                        256 * nh + 128 * t:256 * nh + 128 * t + 128]).astype(F32)
                for kh in range(2) for nh in range(2)]
            for k, v in enumerate([b11 + b22, b12 - b22, b21 - b11, b11 + b12, b21 + b22]):
                r, c = ws_pos(k)
                w2b[r + 16 * i:r + 16 * (i + n), c + 128 * t:c + 128 * t + 128] = v.astype(BF16)

    def mix(r0, r1, t, bt):
        pos = [AT * t + AS * (2 * ((r % 1024) // 16) + r // 1024) for r in range(r0, r1, 16)]
        at = jnp.concatenate([a_ref[p:p + 16, :] for p in pos], axis=0)
        ob[r0:r1, 128 * t:128 * (t + 1)] = (bt + gate[r0:r1, :] * (at - bt)).astype(BF16)

    def out_copy(r0, r1, c0, c1):
        cp = group(0, [(ob.at[pl.ds(r0, r1 - r0), pl.ds(c0, c1 - c0)],
                        o_hbm.at[pl.ds(r0, r1 - r0), pl.ds(c0, c1 - c0)])])
        start(cp)
        return cp

    def mm2(r0, r1):
        q0, q1 = 1024 + r0, 1024 + r1

        def a_blk(lo, hi, nts):
            return jnp.concatenate([_bf(actw[nt, lo // 2:hi // 2, :]) for nt in nts], axis=1)

        def ws(k):
            r, c = ws_pos(k)
            return _bf(w2s[r // 2:r // 2 + 320, c:c + 256])

        def dot(a, b):
            return jnp.dot(a, b, preferred_element_type=F32)

        a11, a12 = a_blk(r0, r1, range(0, 5)), a_blk(r0, r1, range(5, 10))
        a21, a22 = a_blk(q0, q1, range(0, 5)), a_blk(q0, q1, range(5, 10))
        b11 = _bf(w2s[0:320, 0:256])
        b22 = _bf(w2s[320:640, 256:512])
        wl = _bf(w2s[640:704, :])
        e1 = dot(a_blk(r0, r1, (10,)), wl)
        e2 = dot(a_blk(q0, q1, (10,)), wl)
        cps = []
        m3 = dot(a11, ws(1))
        m5 = dot(addbf(a11, a12, 1), b22)
        last = r1 == 1024
        c12 = m3 + m5 + e1[:, 256:512]
        for t in range(2):
            mix(r0, r1, 2 + t, c12[:, 128 * t:128 * (t + 1)])
        if last:
            cps += out_copy(r0, r1, 256, 512)
        m4 = dot(a22, ws(2))
        m2 = dot(addbf(a21, a22, 1), b11)
        c21 = m2 + m4 + e2[:, 0:256]
        for t in range(2):
            mix(q0, q1, t, c21[:, 128 * t:128 * (t + 1)])
        if last:
            cps += out_copy(q0, q1, 0, 256)
        m1 = dot(addbf(a11, a22, 1), ws(0))
        m7 = dot(addbf(a12, a22, -1), ws(4))
        c11 = (m4 - m5 + e1[:, 0:256]) + m1 + m7
        for t in range(2):
            mix(r0, r1, t, c11[:, 128 * t:128 * (t + 1)])
        cps += out_copy(r0, r1, 0, 256 if last else D)
        m6 = dot(addbf(a21, a11, -1), ws(3))
        c22 = (m3 - m2 + e2[:, 256:512] + m1) + m6
        for t in range(2):
            mix(q0, q1, 2 + t, c22[:, 128 * t:128 * (t + 1)])
            if last:
                cps += out_copy(q0, q1, 256 + 128 * t, 384 + 128 * t)
        if not last:
            cps += out_copy(q0, q1, 0, D)
        return cps, m1

    def tok(v):
        t_a[0, 0, pl.ds(136 + z, 8), :] = v

    def tok_b(v):
        t_b[0, 0, pl.ds(136 + z, 8), :] = v

    def tok_u(v):
        u_ref[pl.ds(16 * UB + z, 8), :] = pltpu.bitcast(v, U32)

    def tok_act(v):
        actw[NF + z, 0:8, :] = v

    def tok_w(v):
        w2s[pl.ds(pl.multiple_of(WS_END + 8 * z, 8), 8), 0:128] = pltpu.bitcast(v, U32)

    def paced(units, chains, tail=128):
        res = [u() for u in units]
        cap = [(SW if d == 896 else 1.0) for d, _ in res]
        total = sum(d * c for (d, _), c in zip(res, cap))

        def token(t):
            for (d, fn), c in zip(res, cap):
                if t < d * c:
                    return fn(min(int(t / c), d - 1))
                t -= d * c
        ev = []
        for ci, (tk, jobs, f0, f1_) in enumerate(chains):
            t0, t1 = f0 * (total - tail), f1_ * (total - tail)
            for n, job in enumerate(jobs):
                ev.append((int(t0 + n * (t1 - t0) / len(jobs)), ci, n, tk, job))
        ev.sort(key=lambda e: e[:3])
        for t, _, _, tk, job in ev:
            tk(token(t))
            job()

    def U(fn, *a):
        return lambda: fn(*a)

    def f1_jobs(i, ps=range(8)):
        return [U(f1, i, (p,)) for p in ps]

    def x_chain(p, f0, f1_):
        def tk(v):
            xsumw[p][10 + z, 0:8, :] = pltpu.bitcast(v, U32)
        return (tk, [U(x_mini, p, i, 2) for i in range(0, 16, 2)], f0, f1_)

    def w_chain(tp, f0, f1_):
        def tk(v):
            wsumw[tp][10 + z, 0:8, :] = pltpu.bitcast(v, U32)
        return (tk, [U(w1_mini, tp, i, 2) for i in range(0, 8, 2)], f0, f1_)

    wait(d0)
    start(d2)
    z = one_ref[0] - 1
    mm1((0,), 0)
    wait(d1)
    start(d3)
    paced([U(mm1, (0,), 1), U(mm1, (4,), 0), U(mm1, (4,), 1)], [(tok_u, f1_jobs(0, range(4)), 0, 1)])
    wait(d2)
    start(d4)
    start(d5)
    paced([U(mm1, (1,), 0), U(mm1, (1,), 1), U(mm1, (0, 4, 1), 2), U(mm1, (0, 4, 1), 3)],
          [(tok_u, f1_jobs(0, range(4, 8)), 0, 1), x_chain(0, 0.08, 1.0), w_chain(0, 0.14, 0.6), w_chain(1, 0.64, 1.0)])
    wait(d3)
    paced([U(mm1, (5,), nt) for nt in range(4)], [x_chain(2, 0, 0.8), w_chain(2, 0.05, 1.0)])
    paced([U(mm1s, 2, 0), U(mm1s, 2, 1), U(mm1s, 0, 2)],
          [(tok_u, f1_jobs(1) + f1_jobs(2, range(F1S)), 0, 1), x_chain(1, 0.04, 1.0)])
    wait(d4)
    gw = gws[...].reshape(1, D).astype(F32)
    rowp = lax.broadcasted_iota(jnp.int32, (FP - F, D), 0)
    padv = _u32(jnp.where(rowp == 0, jnp.broadcast_to(gw, (FP - F, D)), 0.0).astype(BF16))
    w1s[F // 2:FP // 2, :] = padv
    paced([U(mm1s, 2, 2), U(mm1s, 1, 2)],
          [(tok_u, f1_jobs(2, range(F1S, 8)) + f1_jobs(3, range(F1T)), 0, 1), x_chain(3, 0.05, 0.9)])
    paced([U(mm1s, 3, 0)], [(tok_u, f1_jobs(3, range(F1T, 8)), 0, 1)], tail=450)

    pend = []
    deps = {}
    for s_lo in range(16 + LAG):
        if s_lo < 16:
            pend.append(phase_a1(s_lo, deps.get(s_lo)))
        if 2 <= s_lo and s_lo + DA < 16:
            deps[s_lo + DA] = t_a[1, 0, pl.ds(136 + z, 8), :] + t_b[1, 0, pl.ds(136 + z, 8), :]
        if s_lo == 8:
            special()
        if s_lo == 16:
            mm1s(3, 1)
        if s_lo >= LAG:
            phase_a2(s_lo - LAG, *pend[s_lo - LAG])

    def both(*jobs):
        def run():
            for fn, r0, a in jobs:
                fn(r0, a)
        return run

    def make_slots(rgs):
        slots = [both((p1, rgs[0], 0), (p1, rgs[0], 1)), both((p1, rgs[0], 2), (p1, rgs[0], 3))]
        late = [(p1, r, a) for r in rgs[1:] for a in range(4)]
        p3q, done = [], set()
        for j in range(len(rgs)):
            for a in range(4):
                slots.append(both((p2, rgs[j], a)))
                if late and (a % 2 == 1 or not p3q):
                    slots.append(both(late.pop(0), late.pop(0)))
                elif p3q:
                    slots.append(both(p3q.pop(0)))
            done.add(rgs[j])
            base = rgs[j] - rgs[j] % 16
            if rgs[j] != 256 and base in done and base + 8 in done:
                p3q += [(p3, base, a) for a in range(4)]
        assert not late
        return slots + [both(job) for job in p3q]

    mm1s(3, 2)
    wait(d5)
    sl_a = make_slots([8 * i for i in range(2, 16)] + [256, 8, 0])
    sl_b = make_slots([8 * i for i in range(16, 32)])

    su = [(p, tp) for tp in (3, 4) for p in range(4)]
    std = [U(mm1, (2 * q, 2 * q + 1), 10) for q in range(4)]
    std += [U(mm1, (p, p + 4), 2 * tp + o) for p, tp in su[NSB:] for o in range(2)]
    strs = [U(mm1s, p, tp) for p, tp in su[:NSB]]
    tot = 512 * len(std) + 896 * SW * len(strs)
    na, nb = int(len(sl_a) * 1024 / (tot - BT)), int(len(sl_b) * 1024 / (tot - BT))
    wch = [w_chain(tp, 0.1, 0.9) for tp in (3, 4) if any(t == tp for _, t in su[:NSB])]
    paced(std[0:2], [(tok, sl_a[:na], 0, 1), (tok_b, sl_b[:nb], 0.5 / nb, 1 + 0.49 / nb)] + wch, tail=0)
    bu = std[2:] + strs
    hb = 0.5 / len(sl_b[nb:])
    paced(bu, [(tok, sl_a[na:], 0, 1), (tok_b, sl_b[nb:], hb, 1 + hb), (tok_w, [U(w2_mini, n, 1) for n in range(40)], 0.03, 0.97)], tail=BT)

    pend = []
    zs = {}
    for s_lo in range(17):
        if s_lo < 16:
            pend.append(phase_c1(s_lo, zs[s_lo - DC - 1][0:4] if s_lo - DC - 1 >= 0 else None))
        if s_lo >= 1:
            sg = s_lo - 1
            zs[sg] = phase_c2(sg, zs[sg - DC][4:8] if sg - DC >= 0 else None, sg + DC < 16, *pend[sg])

    outs = []
    tok_act(pend[TOKC][0][0:8])
    for r0, r1 in MM2_CHUNKS:
        cps, m1 = mm2(r0, r1)
        outs += cps
        if r1 != 1024:
            tok_act(pltpu.bitcast(m1[0:8, 0:128], U32))
    wait(outs)


@jax.jit
def pallas_gated_mix__spectral_gfnet__dense_activation_silu__prompt_kernel(A_x, A_w_r, A_w_i, B_x, B_w1, B_w2, gate_w):
    small, g = _consts()
    out = pl.pallas_call(
        _kernel,
        out_shape=jax.ShapeDtypeStruct((S, D), BF16),
        in_specs=[pl.BlockSpec(memory_space=pl.ANY)] * 9,
        out_specs=pl.BlockSpec(memory_space=pl.ANY),
        scratch_shapes=[
            pltpu.VMEM((S // 2, D), U32),
            pltpu.VMEM((128, S), U32),
            pltpu.VMEM((128, S), U32),
            pltpu.VMEM((1, S), BF16),
            pltpu.VMEM((1, S), BF16),
            pltpu.VMEM((16, S), BF16),
            pltpu.VMEM((16, S), BF16),
            pltpu.VMEM((FP // 2, D), U32),
            pltpu.VMEM((WS_END + 8, D), U32),
            pltpu.VMEM((D,), BF16),
            pltpu.VMEM((O_END, 128), U32),
            pltpu.VMEM((32, 64, 128), U32),
            pltpu.VMEM((18 * UB, 128), U32),
            pltpu.VMEM((16, 2, 144, 128), F32),
            pltpu.VMEM((16, 2, 144, 128), F32),
            pltpu.VMEM((16, 2, 256, 128), BF16),
            pltpu.VMEM((4 * AT + 32, 128), F32),
            pltpu.VMEM((8, S), F32),
            pltpu.VMEM((NF + 1, S, 128), BF16),
            pltpu.VMEM((S, 128), F32),
            pltpu.VMEM((S, D), BF16),
            *[pltpu.VMEM((11, 256, 128), BF16)] * 4,
            *[pltpu.VMEM((11, 128, 128), BF16)] * 5,
            pltpu.SMEM((128,), jnp.int32),
            pltpu.SemaphoreType.DMA((3,)),
        ],
        compiler_params=pltpu.CompilerParams(vmem_limit_bytes=100 * 1024 * 1024),
    )(jnp.asarray(np.arange(1, 129, dtype=np.int32)), A_x[0], A_w_r.T, A_w_i.T, B_w1.T, B_w2, gate_w, jnp.asarray(small), jnp.asarray(g))
    return out[None]
```

```python
import numpy as np
import jax
import jax.numpy as jnp
from jax import lax
import jax.experimental.pallas as pl
import jax.experimental.pallas.tpu as pltpu

S, D, F = 2048, 512, 1376
FP = 1408
NF = 11
NT = (((1,), (1,)), ((), ()))
AS = 20
AT = AS * 128 + 8
UB = 258
WS_END = 704 + 960
MM2_CHUNKS = [(0, 256), (256, 512), (512, 768), (768, 896), (896, 1024)]
LAG, DA, DC, TOKC, GR = 1, 2, 2, 15, 32
SW, NSB, BT, F1S, F1T, P1_EARLY, VT, UT, NH = 0.8, 8, 900, 4, 5, 3, 520, 600, 6
HQ = float(np.sqrt(0.5))
F32 = jnp.float32
BF16 = jnp.bfloat16
U32 = jnp.uint32

O_LD0, O_LD2, O_LDA, O_LDB, O_RD0, O_RD2, O_RDA, O_RDB, O_J, O_END = 0, 72, 136, 200, 264, 328, 392, 456, 520, 584


def _pack_rows(a):
    f = np.ascontiguousarray(a, dtype=np.float32)
    u = f.view(np.uint32).astype(np.uint64)
    b = ((u + 0x7FFF + ((u >> 16) & 1)) >> 16).astype(np.uint32)
    return (b[..., 0::2, :] | (b[..., 1::2, :] << 16)).astype(np.uint32)


def _consts():
    n2 = np.arange(128)
    j = np.arange(64)
    ld0 = np.zeros((144, 128))
    th = 2 * np.pi * np.outer(4 * j, n2) / 512
    ld0[0:64] = np.cos(th)
    ld0[64:128] = -np.sin(th)
    ld0[128] = np.cos(np.pi * n2)
    ld2 = np.zeros((128, 128))
    th = 2 * np.pi * np.outer(4 * j + 2, n2) / 512
    ld2[0:64] = np.cos(th)
    ld2[64:128] = -np.sin(th)
    i = np.arange(128)
    th = 2 * np.pi * np.outer(2 * i + 1, n2) / 512
    sg = np.where(i % 2 == 0, -1.0, 1.0)[:, None]
    ld1 = np.zeros((256, 256))
    ld1[0:128, 0:128] = np.cos(th)
    ld1[0:128, 128:256] = sg * np.sin(th)
    ld1[128:256, 0:128] = -np.sin(th)
    ld1[128:256, 128:256] = sg * np.cos(th)
    sc = 2.0 / (S * D)
    rd0 = np.zeros((128, 128))
    rd0[0::2] = ld0[0:64] * sc
    rd0[1::2] = ld0[64:128] * sc
    rd0[0] = ld0[0] * sc / 4
    rd0[1] = ld0[128] * sc / 4
    rd2 = np.zeros((128, 128))
    rd2[1::2] = ld2[0:64] * sc
    rd2[(2 * j + 2) % 128] = ld2[64:128] * sc
    hq = np.sqrt(0.5)
    eye, n64 = np.eye(256), np.arange(64)
    p_, q_ = eye[:, 0:128], eye[:, 128:256]
    lo = (np.arange(128) < 64)[None, :]
    e_ = np.where(lo, p_, hq * (p_ + q_))
    c_ = np.where(lo, q_, hq * (p_ - q_))
    r_ = np.roll(c_, 64, axis=1)
    mm = np.concatenate([e_ + r_, e_ - r_], axis=1).T
    ldv = ld1 @ mm.T / 2
    cls_a = (i % 4 == 0) | (i % 4 == 3)
    assert np.abs(ldv[np.concatenate([cls_a, cls_a])][:, 128:]).max() < 1e-9
    assert np.abs(ldv[np.concatenate([~cls_a, ~cls_a])][:, :128]).max() < 1e-9
    sg_ = np.arange(64)
    ia = np.where(sg_ % 2 == 0, 2 * sg_, 2 * sg_ + 1)
    ib = np.where(sg_ % 2 == 0, 2 * sg_ + 1, 2 * sg_)
    lda = np.concatenate([ldv[ia, :128], ldv[128 + ia, :128]], axis=0)
    ldb = np.concatenate([ldv[ib, 128:], ldv[128 + ib, 128:]], axis=0)
    rda, rdb = np.zeros((128, 128)), np.zeros((128, 128))
    ia_, ib_ = i[cls_a], i[~cls_a]
    rda[ia_] = ldv[ia_, :128] * sc
    rda[(ia_ + 2) % 128] = ldv[128 + ia_, :128] * sc
    rdb[ib_] = ldv[ib_, 128:] * sc
    rdb[(ib_ + 2) % 128] = ldv[128 + ib_, 128:] * sc
    e = np.arange(64)
    kl = np.arange(64)
    g = np.zeros((16, 2, 128, 128))
    for s_lo in range(16):
        for kb in range(2):
            th = -2 * np.pi * np.outer(s_lo + 16 * e, 2 * kl + kb) / S
            gr, gi = np.cos(th), np.sin(th)
            if kb == 0:
                rr, ri = slice(0, 64), slice(64, 128)
                cr, ci = 2 * kl, 2 * kl + 1
            else:
                rr, ri = slice(64, 128), slice(0, 64)
                cr, ci = 2 * kl + 1, (2 * kl + 2) % 128
            m = np.zeros((128, 128))
            m[rr, cr] = gr
            m[rr, ci] = gi
            m[ri, cr] = -gi
            m[ri, ci] = gr
            g[s_lo, kb] = m
    jrev = np.zeros((128, 128))
    jrev[np.arange(128), 127 - np.arange(128)] = 1.0
    small = np.concatenate([ld0, ld2, lda, ldb, rd0, rd2, rda, rdb, jrev], axis=0)
    return _pack_rows(small), _pack_rows(g.reshape(32, 128, 128))


def _dft4(z, inv):
    (ar, ai), (br, bi), (cr, ci), (dr, di) = z
    s0r, s0i = ar + cr, ai + ci
    s1r, s1i = ar - cr, ai - ci
    s2r, s2i = br + dr, bi + di
    s3r, s3i = br - dr, bi - di
    y0 = (s0r + s2r, s0i + s2i)
    y2 = (s0r - s2r, s0i - s2i)
    if not inv:
        y1 = (s1r + s3i, s1i - s3r)
        y3 = (s1r - s3i, s1i + s3r)
    else:
        y1 = (s1r - s3i, s1i + s3r)
        y3 = (s1r + s3i, s1i - s3r)
    return [y0, y1, y2, y3]


def _tw16(z, ex, inv):
    r, i = z
    ex = ex % 16
    if ex == 0:
        return z
    sgn = 1.0 if inv else -1.0
    if ex == 4:
        return (-i, r) if inv else (i, -r)
    c = float(np.cos(2 * np.pi * ex / 16))
    s = sgn * float(np.sin(2 * np.pi * ex / 16))
    if ex in (2, 6):
        h = float(np.sqrt(0.5))
        if c > 0 and s > 0:
            return ((r - i) * h, (r + i) * h)
        if c > 0 and s < 0:
            return ((r + i) * h, (i - r) * h)
        if c < 0 and s > 0:
            return ((r + i) * (-h), (r - i) * h)
        return ((i - r) * h, (r + i) * (-h))
    return (r * c - i * s, r * s + i * c)


def _unpack(w, idx):
    bits = (w << 16) if idx == 0 else (w & jnp.uint32(0xFFFF0000))
    return lax.bitcast_convert_type(bits, F32)


def _bf(w):
    return pltpu.bitcast(w, BF16)


def _u32(v):
    return pltpu.bitcast(v, U32)


def _kernel(*refs):
    z = pl.program_id(0)
    pl.when(z == 0)(lambda: _body(z, *refs))


def _body(z, x_hbm, wr_hbm, wi_hbm, w1_hbm, w2_hbm, gw_hbm, sm_hbm, g_hbm,
            o_hbm,
            xs, wrs, wis, nyq_r, nyq_i, dc_r, dc_i, w1s, w2s, gws, sm, gm,
            u_ref, t_a, t_b, v_ref, a_ref, sp_ref, act, gate, lt_ref, e_ref, wls, os_, xs0, xs1, xs2, xs3, wq0, wq1, wq2, wq3, wq4, sem):
    xsum, wsum = (xs0, xs1, xs2, xs3), (wq0, wq1, wq2, wq3, wq4)
    xsumw = [r.bitcast(U32) for r in xsum]
    wsumw = [r.bitcast(U32) for r in wsum]
    lane = lax.broadcasted_iota(jnp.int32, (1, 128), 1)
    lo_half = lane < 64
    even = (lane % 2) == 0
    cls_a = ((lane + 1) % 4) < 2
    row_even = (lax.broadcasted_iota(jnp.int32, (1, 8, 128), 1) % 2) == 0

    xb, w1b, w2b = xs.bitcast(BF16), w1s.bitcast(BF16), w2s.bitcast(BF16)
    wrb, wib = wrs.bitcast(BF16), wis.bitcast(BF16)
    vw, actw, ob = v_ref.bitcast(U32), act.bitcast(U32), os_

    def pk(lo, hi):
        half = jnp.uint32(0x8000)
        lo = (lax.bitcast_convert_type(lo, U32) + half) >> 16
        hi = (lax.bitcast_convert_type(hi, U32) + half) & jnp.uint32(0xFFFF0000)
        return lo | hi

    def group(k, pairs):
        return [pltpu.make_async_copy(s, d, sem.at[k]) for s, d in pairs]

    def start(cps):
        for c in cps:
            c.start()

    def wait(cps):
        for c in cps:
            c.wait()

    def w1_pairs(f0, f1):
        return [(w1_hbm.at[pl.ds(f0, f1 - f0), :], w1b.at[pl.ds(f0, f1 - f0), :])]

    def x_pairs(*blks):
        return [(x_hbm.at[pl.ds(256 * b, 256), :], xb.at[pl.ds(256 * b, 256), :]) for b in blks]

    d0 = group(0, w1_pairs(0, 128) + x_pairs(0) + [(gw_hbm, gws)])
    d1 = group(1, w1_pairs(128, 256) + x_pairs(4))
    d2 = group(0, x_pairs(1) + w1_pairs(256, 512))
    d3 = group(1, x_pairs(5, 2, 6) + w1_pairs(512, 768))
    d4 = group(0, x_pairs(3, 7) + [(sm_hbm, sm), (g_hbm, gm)]
               + [(wr_hbm.at[pl.ds(256, 1), :], nyq_r), (wi_hbm.at[pl.ds(256, 1), :], nyq_i)]
               + [(wr_hbm.at[pl.ds(0, 16), :], dc_r), (wi_hbm.at[pl.ds(0, 16), :], dc_i)])
    d5 = group(2, w1_pairs(768, F)
               + [(wr_hbm.at[pl.ds(0, 256), :], wrb), (wi_hbm.at[pl.ds(0, 256), :], wib.at[:, pl.ds(256, S)])]
               + [(w2_hbm.at[pl.ds(0, 1280), :], w2b.at[pl.ds(0, 1280), :]),
                  (w2_hbm.at[pl.ds(1280, F - 1280), :], wls.bitcast(BF16).at[pl.ds(0, F - 1280), :])])

    for d in (d0, d1):
        start(d)

    w1s[F // 2:FP // 2, :] = jnp.zeros(((FP - F) // 2, D), U32)
    wls[(F - 1280) // 2:64, :] = jnp.zeros(((FP - F) // 2, D), U32)
    t_a[1, 0, 136:144, :] = jnp.zeros((8, 128), F32)
    t_b[1, 0, 136:144, :] = jnp.zeros((8, 128), F32)

    def tloc(r0):
        return (t_b, r0 - 128) if 128 <= r0 < 256 else (t_a, min(r0, 128))
    a_ref[4 * AT:4 * AT + 8, :] = jnp.zeros((8, 128), F32)
    lt_ref[0:16, :] = jnp.zeros((16, 128), F32)

    def after(w, zero):
        return jnp.concatenate([w[0:8] | pltpu.bitcast(zero, U32), w[8:]], axis=0)

    def after4(w, zeros):
        if zeros is None:
            return w
        return jnp.concatenate([after(w[16 * j:16 * j + 16], zeros[j]) for j in range(4)], axis=0)

    def addbf(p, q, sign):
        p, q = p.astype(F32), q.astype(F32)
        return (p + q if sign > 0 else p - q).astype(BF16)

    def silu_store(h, ranges, nt):
        hh = 0.5 * h
        th = jnp.tanh(hh)
        a = (hh + hh * th).astype(BF16)
        off = 0
        for r0, r1 in ranges:
            act[nt, r0:r1, :] = a[off:off + r1 - r0]
            off += r1 - r0

    def ntdot(a, b):
        return lax.dot_general(a, b, NT, preferred_element_type=F32)

    def mm1(bs, nt):
        ranges = [(256 * b, 256 * b + 256) for b in bs]
        x = jnp.concatenate([_bf(xs[r0 // 2:r1 // 2, :]) for r0, r1 in ranges], axis=0)
        h = ntdot(x, _bf(w1s[64 * nt:64 * (nt + 1), :]))
        silu_store(h, ranges, nt)
        return 256 * len(bs), lambda t: h[(t // 8) * 8:(t // 8) * 8 + 8]

    def e_unit(q):
        e = jnp.dot(_bf(actw[NF - 1, 256 * q:256 * q + 256, :]), _bf(wls[...]), preferred_element_type=F32)
        e_ref[512 * q:512 * q + 512, :] = e
        return 512, lambda t: e[(t // 8) * 8:(t // 8) * 8 + 8, 0:128]

    def x_mini(p, i, n):
        for t in range(2):
            a11, a12, a21, a22 = [
                _bf(xs[512 * mh + 128 * p + 8 * i:512 * mh + 128 * p + 8 * (i + n),
                       256 * kh + 128 * t:256 * kh + 128 * t + 128]).astype(F32)
                for mh in range(2) for kh in range(2)]
            for k, v in enumerate([a11 + a22, a21 + a22, a11 + a12, a21 - a11, a12 - a22]):
                xsum[p][2 * k + t, 16 * i:16 * (i + n), :] = v.astype(BF16)

    def w1_mini(tp, i, n):
        for t in range(2):
            b11, b12, b21, b22 = [
                _bf(w1s[128 * tp + 64 * nh + 8 * i:128 * tp + 64 * nh + 8 * (i + n),
                        256 * kh + 128 * t:256 * kh + 128 * t + 128]).astype(F32)
                for kh in range(2) for nh in range(2)]
            for k, v in enumerate([b11 + b22, b12 - b22, b21 - b11, b11 + b12, b21 + b22]):
                wsum[tp][2 * k + t, 16 * i:16 * (i + n), :] = v.astype(BF16)

    def mm1s(p, tp):
        a11 = _bf(xs[128 * p:128 * p + 128, 0:256])
        a22 = _bf(xs[512 + 128 * p:512 + 128 * p + 128, 256:512])
        b11 = _bf(w1s[128 * tp:128 * tp + 64, 0:256])
        b22 = _bf(w1s[128 * tp + 64:128 * tp + 128, 256:512])
        sa = [jnp.concatenate([_bf(xsumw[p][2 * k, 0:128, :]), _bf(xsumw[p][2 * k + 1, 0:128, :])], axis=1) for k in range(5)]
        sb = [jnp.concatenate([_bf(wsumw[tp][2 * k, 0:64, :]), _bf(wsumw[tp][2 * k + 1, 0:64, :])], axis=1) for k in range(5)]
        top, bot = [(256 * p, 256 * p + 256)], [(1024 + 256 * p, 1024 + 256 * p + 256)]
        m3 = ntdot(a11, sb[1])
        m5 = ntdot(sa[2], b22)
        silu_store(m3 + m5, top, 2 * tp + 1)
        m4 = ntdot(a22, sb[2])
        m2 = ntdot(sa[1], b11)
        silu_store(m2 + m4, bot, 2 * tp)
        m1 = ntdot(sa[0], sb[0])
        m7 = ntdot(sa[4], sb[4])
        silu_store((m4 - m5) + m1 + m7, top, 2 * tp)
        m6 = jnp.concatenate([ntdot(sa[3][0:128], sb[3]), ntdot(sa[3][128:256], sb[3])], axis=0)
        silu_store((m3 - m2 + m1) + m6, bot, 2 * tp + 1)
        ms = (m3, m4, m1, m6)
        return 896, lambda t: ms[t // 256][((t % 256) // 8) * 8:((t % 256) // 8) * 8 + 8]

    def f1(i, ps=range(8)):
        for p in ps:
            ew = 8 * i + p
            w = [[xs[512 * c + 16 * ew + 8 * o:512 * c + 16 * ew + 8 * o + 8, :] for c in range(2)]
                 for o in range(2)]
            for h in range(2):
                outs = []
                for o in range(2):
                    x0, x1 = _unpack(w[o][0], h), _unpack(w[o][1], h)
                    res = []
                    for zz in (x0 + x1, x0 - x1):
                        y0, y1, y2, y3 = [zz[:, 128 * t:128 * (t + 1)] for t in range(4)]
                        a0, a1 = y0 + y2, y1 + y3
                        pp, qq = y0 - y2, y1 - y3
                        ee = jnp.where(lo_half, pp, HQ * (pp + qq))
                        rr = pltpu.roll(jnp.where(lo_half, qq, HQ * (pp - qq)), 64, 1)
                        res.append((a0 + a1, a0 - a1, ee + rr, ee - rr))
                    outs.append(res)
                for kb in range(2):
                    for t in range(4):
                        u_ref[pl.ds(UB * h + 64 * t + 32 * kb + ew, 8, stride=2 * UB), :] = pk(
                            outs[0][kb][t], outs[1][kb][t])

    def phase_a1(s_lo, dep):
        u = [u_ref[UB * s_lo + 64 * t:UB * s_lo + 64 * t + 64, :] for t in range(4)]
        if dep is not None:
            u[0] = after(u[0], dep)
        u = [_bf(w) for w in u]
        o0 = lax.dot_general(_bf(sm[O_LD0:O_LD2, :]), u[0], NT, preferred_element_type=F32)
        o2 = lax.dot_general(_bf(sm[O_LD2:O_LDA, :]), u[1], NT, preferred_element_type=F32)
        oa = lax.dot_general(_bf(sm[O_LDA:O_LDB, :]), u[2], NT, preferred_element_type=F32)
        ob_ = lax.dot_general(_bf(sm[O_LDB:O_RD0, :]), u[3], NT, preferred_element_type=F32)
        r_e = pk(o0[0:64], o2[0:64])
        i_e = pk(o0[64:128], o2[64:128])
        oa, ob_ = oa.reshape(16, 8, 128), ob_.reshape(16, 8, 128)
        od = pk(jnp.where(row_even, oa, ob_).reshape(128, 128), jnp.where(row_even, ob_, oa).reshape(128, 128))
        r_o, i_o = od[0:64], od[64:128]
        r_n = pk(o0[128:136], o0[136:144])
        zero = jnp.zeros_like(r_n)
        r = jnp.concatenate([r_e, r_o], axis=0)
        t = pltpu.roll(jnp.concatenate([i_e, i_o], axis=0), 64, 1)
        la = _bf(jnp.concatenate([jnp.where(lo_half, r, t), jnp.where(lo_half, r_n, zero)], axis=0))
        lb = _bf(jnp.concatenate([jnp.where(lo_half, t, r), jnp.where(lo_half, zero, r_n)], axis=0))
        return (la, lb), [o0[0:8], o0[64:72]]

    def phase_a2(s_lo, la, lb):
        oa = jnp.dot(la, _bf(gm[2 * s_lo]), preferred_element_type=F32)[0:264]
        ob_ = jnp.dot(lb, _bf(gm[2 * s_lo + 1]), preferred_element_type=F32)[0:264]
        for ri, v in enumerate((jnp.where(even, oa, ob_), pltpu.roll(jnp.where(even, ob_, oa), 127, 1))):
            t_a[s_lo, ri, 0:128, :] = v[0:128]
            t_b[s_lo, ri, 0:128, :] = v[128:256]
            t_a[s_lo, ri, 128:136, :] = v[256:264]
        return [oa[0:8], oa[128:136]]

    row8 = lax.broadcasted_iota(jnp.int32, (8, 128), 0)

    def special():
        row = lax.broadcasted_iota(jnp.int32, (16, S), 0)

        def rowcat(ref):
            return jnp.broadcast_to(
                ref[0:1, :].astype(F32), (16, S))
        q = jnp.where(row == 0, rowcat(dc_r),
            jnp.where(row == 1, rowcat(dc_i),
            jnp.where(row == 2, jnp.broadcast_to(nyq_r[...].astype(F32), (16, S)),
            jnp.where(row == 3, jnp.broadcast_to(nyq_i[...].astype(F32), (16, S)), 0.0))))
        qb = q.astype(BF16)
        stacked = jnp.concatenate([qb[:, 128 * (15 - t):128 * (16 - t)] for t in range(16)], axis=0)
        rv = jnp.dot(stacked, _bf(sm[O_J:O_END, :]), preferred_element_type=F32)
        rev = jnp.concatenate([rv[16 * t:16 * t + 8] for t in range(16)], axis=1)
        mir = pltpu.roll(rev, 1, 1)
        sgn = jnp.where((lax.broadcasted_iota(jnp.int32, (8, S), 0) % 2) == 0, 1.0, -1.0)
        sp_ref[...] = q[0:8] + sgn * mir

    def ld(s, r0, n=8):
        ref, r = tloc(r0)
        return ref[s, 0, r:r + n, :], ref[s, 1, r:r + n, :]

    def st(s, r0, z):
        ref, r = tloc(r0)
        ref[s, 0, r:r + 8, :] = z[0]
        ref[s, 1, r:r + 8, :] = z[1]

    def sp_row(r, kt, other):
        return jnp.where(row8 == 0, jnp.broadcast_to(sp_ref[r:r + 1, 128 * kt:128 * (kt + 1)], (8, 128)), other)

    def p1(r0, n2):
        y = _dft4([ld(4 * n1 + n2, r0) for n1 in range(4)], False)
        for k1 in range(4):
            st(4 * k1 + n2, r0, _tw16(y[k1], k1 * n2, False))

    def p2(r0, k1):
        y = _dft4([ld(4 * k1 + n2, r0) for n2 in range(4)], False)
        u = []
        for k2 in range(4):
            kt = k1 + 4 * k2
            if r0 == 256:
                wr, wi = sp_row(2, kt, 0.0), sp_row(3, kt, 0.0)
            else:
                i8, h = r0 % 128, r0 // 128
                sl = slice(128 * kt, 128 * (kt + 1))
                rows = pl.ds(i8, 8) if h == 0 else pl.ds(pl.multiple_of(i8 + 8 * z, 8), 8)
                wr, wi = _unpack(wrs[rows, sl], h), _unpack(wis[rows, 128 * kt + 256:128 * kt + 384], h)
                if r0 == 0:
                    wr, wi = sp_row(0, kt, wr), sp_row(1, kt, wi)
            xr, xi = y[k2]
            ur, ui = xr * wr - xi * wi, xr * wi + xi * wr
            if r0 == 0:
                er, ei = ld(4 * k1 + k2, 256)
                ur, ui = ur - ei, ui + er
            u.append((ur, ui))
        if r0 == 256:
            for k2 in range(4):
                st(4 * k1 + k2, r0, u[k2])
            return
        y = _dft4(u, True)
        for n2 in range(4):
            st(4 * k1 + n2, r0, _tw16(y[n2], k1 * n2, True))

    def p3(r0, n2):
        y = _dft4([ld(4 * k1 + n2, r0, 16) for k1 in range(4)], True)
        for n1 in range(4):
            v_ref[4 * n1 + n2, 0, r0:r0 + 16, :] = y[n1][0].astype(BF16)
            v_ref[4 * n1 + n2, 1, r0:r0 + 16, :] = y[n1][1].astype(BF16)

    def phase_c1(s_lo, dep):
        vr = vw[s_lo, 0, 0:128, :]
        t = pltpu.roll(vw[s_lo, 1, 0:128, :], 1, 1)
        va = _bf(jnp.where(even, vr, t))
        vb = _bf(jnp.where(even, t, vr))
        za = lax.dot_general(_bf(after4(gm[2 * s_lo], dep)), va, NT, preferred_element_type=F32)
        zb = lax.dot_general(_bf(gm[2 * s_lo + 1]), vb, NT, preferred_element_type=F32)
        zr = pk(za[0:64] + zb[64:128], za[0:64] - zb[64:128])
        zi = pk(za[64:128] + zb[0:64], za[64:128] - zb[0:64])
        re = zr[:, 0:128]
        t = pltpu.roll(zi[:, 0:128], 1, 1)
        l0 = jnp.where(even, re, t)
        l2 = _bf(jnp.where(even, t, re))
        ro = zr[:, 128:256]
        t = pltpu.roll(zi[:, 128:256], 2, 1)
        la = _bf(jnp.where(cls_a, ro, t))
        lb = _bf(jnp.where(cls_a, t, ro))
        return l0, l2, la, lb

    def phase_c2(s_lo, dep, want, l0, l2, la, lb):
        a0 = jnp.dot(_bf(after4(l0, dep)), _bf(sm[O_RD0:O_RD2, :]), preferred_element_type=F32)
        a2 = jnp.dot(l2, _bf(sm[O_RD2:O_RDA, :]), preferred_element_type=F32)
        va = jnp.dot(la, _bf(sm[O_RDA:O_RDB, :]), preferred_element_type=F32)
        vb = jnp.dot(lb, _bf(sm[O_RDB:O_J, :]), preferred_element_type=F32)
        ee = va + vb
        cc = pltpu.roll(va - vb, 64, 1)
        pp = jnp.where(lo_half, ee, HQ * (ee + cc))
        qq = jnp.where(lo_half, cc, HQ * (ee - cc))
        e0, e1 = a0 + a2, a0 - a2
        ys = [e0 + pp, e1 + qq, e0 - pp, e1 - qq]
        zeros = []
        for k in range(8):
            for t, y in enumerate(ys):
                a_ref[pl.ds(AT * t + s_lo + 16 * k * AS, 16, stride=AS), :] = y[16 * k:16 * k + 16]
            if want:
                zeros.append(a_ref[pl.ds(4 * AT + z, 8), :])
        return zeros

    def ws_pos(k):
        return FP + 640 * (k // 2), 256 * (k % 2)

    def w2_mini(i, n):
        for t in range(2):
            b11, b12, b21, b22 = [
                _bf(w2s[320 * kh + 8 * i:320 * kh + 8 * (i + n),
                        256 * nh + 128 * t:256 * nh + 128 * t + 128]).astype(F32)
                for kh in range(2) for nh in range(2)]
            for k, v in enumerate([b11 + b22, b12 - b22, b21 - b11, b11 + b12, b21 + b22]):
                r, c = ws_pos(k)
                w2b[r + 16 * i:r + 16 * (i + n), c + 128 * t:c + 128 * t + 128] = v.astype(BF16)

    def rnd(v):
        return v.astype(BF16).astype(F32)

    def gate1(r0, r1):
        gw = gws[...].reshape(1, D).astype(F32)
        prod = rnd(_bf(xs[r0 // 2:r1 // 2, :]).astype(F32) * gw)
        part = (prod[:, 0:128] + prod[:, 128:256]) + (prod[:, 256:384] + prod[:, 384:512])
        tot = jnp.sum(part, axis=1, keepdims=True)
        for r in range(r0, r1, 16):
            lt_ref[0:16, r // 16:r // 16 + 1] = tot[r - r0:r - r0 + 16]

    def gate2(c):
        r0, r1 = MM2_CHUNKS[c]
        den = rnd(1.0 + rnd(jnp.exp(-rnd(lt_ref[0:16, :]))))
        g = rnd(1.0 / den)
        om = rnd(1.0 - g)
        for o in (0, 1024):
            for r in range(o + r0, o + r1, 16):
                j = r // 16
                gate[0, r:r + 16, :] = jnp.broadcast_to(g[:, j:j + 1], (16, 128))
                gate[1, r:r + 16, :] = jnp.broadcast_to(om[:, j:j + 1], (16, 128))

    def gate_jobs(c):
        r0, r1 = MM2_CHUNKS[c]
        return [U(gate1, o + r, o + r + GR) for r in range(r0, r1, GR) for o in (0, 1024)]

    def mix(r0, r1, t, bt):
        pos = [AT * t + AS * (2 * ((r % 1024) // 16) + r // 1024) for r in range(r0, r1, 16)]
        at = jnp.concatenate([a_ref[p:p + 16, :] for p in pos], axis=0)
        ob[r0:r1, 128 * t:128 * (t + 1)] = (gate[0, r0:r1, :] * at + gate[1, r0:r1, :] * bt).astype(BF16)

    def out_copy(r0, r1, c0, c1):
        cp = group(0, [(ob.at[pl.ds(r0, r1 - r0), pl.ds(c0, c1 - c0)],
                        o_hbm.at[pl.ds(r0, r1 - r0), pl.ds(c0, c1 - c0)])])
        start(cp)
        return cp

    def mm2(r0, r1):
        q0, q1 = 1024 + r0, 1024 + r1

        def a_blk(lo, hi, nts):
            return jnp.concatenate([_bf(actw[nt, lo // 2:hi // 2, :]) for nt in nts], axis=1)

        def ws(k):
            r, c = ws_pos(k)
            return _bf(w2s[r // 2:r // 2 + 320, c:c + 256])

        def dot(a, b):
            return jnp.dot(a, b, preferred_element_type=F32)

        a11, a12 = a_blk(r0, r1, range(0, 5)), a_blk(r0, r1, range(5, 10))
        a21, a22 = a_blk(q0, q1, range(0, 5)), a_blk(q0, q1, range(5, 10))
        b11 = _bf(w2s[0:320, 0:256])
        b22 = _bf(w2s[320:640, 256:512])
        e1 = e_ref[pl.ds(pl.multiple_of(r0 + 8 * z, 8), r1 - r0), :]
        e2 = e_ref[pl.ds(pl.multiple_of(q0 + 8 * z, 8), r1 - r0), :]
        cps = []
        m3 = dot(a11, ws(1))
        m5 = dot(addbf(a11, a12, 1), b22)
        last = r1 == 1024
        c12 = m3 + m5 + e1[:, 256:512]
        for t in range(2):
            mix(r0, r1, 2 + t, c12[:, 128 * t:128 * (t + 1)])
        if last:
            cps += out_copy(r0, r1, 256, 512)
        m4 = dot(a22, ws(2))
        m2 = dot(addbf(a21, a22, 1), b11)
        c21 = m2 + m4 + e2[:, 0:256]
        for t in range(2):
            mix(q0, q1, t, c21[:, 128 * t:128 * (t + 1)])
        if last:
            cps += out_copy(q0, q1, 0, 256)
        m1 = dot(addbf(a11, a22, 1), ws(0))
        m7 = dot(addbf(a12, a22, -1), ws(4))
        c11 = (m4 - m5 + e1[:, 0:256]) + m1 + m7
        for t in range(2):
            mix(r0, r1, t, c11[:, 128 * t:128 * (t + 1)])
        cps += out_copy(r0, r1, 0, 256 if last else D)
        m6 = dot(addbf(a21, a11, -1), ws(3))
        c22 = (m3 - m2 + e2[:, 256:512] + m1) + m6
        for t in range(2):
            mix(q0, q1, 2 + t, c22[:, 128 * t:128 * (t + 1)])
            if last:
                cps += out_copy(q0, q1, 256 + 128 * t, 384 + 128 * t)
        if not last:
            cps += out_copy(q0, q1, 0, D)
        h = (r1 - r0) // 2
        return cps, m1, [m[r:r + 8, 128 * t:128 * t + 128] for m in (m3, m5, m4, m2, m1) for t in range(2) for r in (0, h)]

    def tok(v):
        t_a[0, 0, pl.ds(136 + z, 8), :] = v

    def tok_b(v):
        t_b[0, 0, pl.ds(136 + z, 8), :] = v

    def tok_u(v):
        u_ref[pl.ds(16 * UB + z, 8), :] = pltpu.bitcast(v, U32)

    def tok_act(v):
        actw[NF + z, 0:8, :] = v

    def tok_g(v):
        lt_ref[pl.ds(16 + z, 8), :] = v

    def tok_x(v):
        xs[pl.ds(pl.multiple_of(S // 2 + 8 * z, 8), 8), 0:128] = pltpu.bitcast(v, U32)

    def tok_w(v):
        w2s[pl.ds(pl.multiple_of(WS_END + 8 * z, 8), 8), 0:128] = pltpu.bitcast(v, U32)

    def paced(units, chains, tail=128):
        res = [u() for u in units]
        cap = [(SW if d == 896 else 1.0) for d, _ in res]
        total = sum(d * c for (d, _), c in zip(res, cap))

        def token(t):
            for (d, fn), c in zip(res, cap):
                if t < d * c:
                    return fn(min(int(t / c), d - 1))
                t -= d * c
        ev = []
        for ci, (tk, jobs, f0, f1_) in enumerate(chains):
            t0, t1 = f0 * (total - tail), f1_ * (total - tail)
            for n, job in enumerate(jobs):
                ev.append((int(t0 + n * (t1 - t0) / len(jobs)), ci, n, tk, job))
        ev.sort(key=lambda e: e[:3])
        for t, _, _, tk, job in ev:
            tk(token(t))
            job()
        return res

    def U(fn, *a):
        return lambda: fn(*a)

    def f1_jobs(i, ps=range(8)):
        return [U(f1, i, (p,)) for p in ps]

    def x_chain(p, f0, f1_):
        def tk(v):
            xsumw[p][10 + z, 0:8, :] = pltpu.bitcast(v, U32)
        return (tk, [U(x_mini, p, i, 2) for i in range(0, 16, 2)], f0, f1_)

    def w_chain(tp, f0, f1_):
        def tk(v):
            wsumw[tp][10 + z, 0:8, :] = pltpu.bitcast(v, U32)
        return (tk, [U(w1_mini, tp, i, 2) for i in range(0, 8, 2)], f0, f1_)

    wait(d0)
    start(d2)
    mm1((0,), 0)
    wait(d1)
    start(d3)
    paced([U(mm1, (0,), 1), U(mm1, (4,), 0), U(mm1, (4,), 1)], [(tok_u, f1_jobs(0, range(4)), 0, 1)])
    wait(d2)
    start(d4)
    start(d5)
    paced([U(mm1, (1,), 0), U(mm1, (1,), 1), U(mm1, (0, 4, 1), 2), U(mm1, (0, 4, 1), 3)],
          [(tok_u, f1_jobs(0, range(4, 8)), 0, 1), x_chain(0, 0.08, 1.0), w_chain(0, 0.14, 0.6), w_chain(1, 0.64, 1.0),
           (tok_g, gate_jobs(0), 0.03, 0.9)])
    wait(d3)
    paced([U(mm1, (5,), nt) for nt in range(4)], [x_chain(2, 0, 0.8), w_chain(2, 0.05, 1.0)])
    paced([U(mm1s, 2, 0), U(mm1s, 2, 1), U(mm1s, 0, 2)],
          [(tok_u, f1_jobs(1) + f1_jobs(2, range(F1S)), 0, 1), x_chain(1, 0.04, 1.0)])
    wait(d4)
    paced([U(mm1s, 2, 2), U(mm1s, 1, 2)],
          [(tok_u, f1_jobs(2, range(F1S, 8)) + f1_jobs(3, range(F1T)), 0, 1), x_chain(3, 0.05, 0.9)])
    res_f = paced([U(mm1s, 3, 0)], [(tok_u, f1_jobs(3, range(F1T, 8)), 0, 1)], tail=450)
    tok_u(res_f[-1][1](UT))

    pend = []
    deps = {}
    for s_lo in range(16 + LAG):
        if s_lo < 16:
            pend.append(phase_a1(s_lo, deps.get(s_lo))[0])
        if 2 <= s_lo and s_lo + DA < 16:
            deps[s_lo + DA] = t_a[1, 0, pl.ds(136 + z, 8), :] + t_b[1, 0, pl.ds(136 + z, 8), :]
        if s_lo == 8:
            special()
        if s_lo == 4:
            gate2(0)
        if s_lo == 16:
            mm1s(3, 1)
        if s_lo >= LAG:
            phase_a2(s_lo - LAG, *pend[s_lo - LAG])

    def both(*jobs):
        def run():
            for fn, r0, a in jobs:
                fn(r0, a)
        return run

    def make_slots(rgs, ne):
        early = [both((p1, r, a), (p1, r, a + 1)) for r in rgs[:ne] for a in (0, 2)]
        slots = []
        late = [(p1, r, a) for r in rgs[ne:] for a in range(4)]
        p3q, done = [], set()
        for j in range(len(rgs)):
            for a in range(4):
                slots.append(both((p2, rgs[j], a)))
                if late and (a % 2 == 1 or not p3q):
                    slots.append(both(late.pop(0), late.pop(0)))
                elif p3q:
                    slots.append(both(p3q.pop(0)))
            done.add(rgs[j])
            base = rgs[j] - rgs[j] % 16
            if rgs[j] != 256 and base in done and base + 8 in done:
                p3q += [(p3, base, a) for a in range(4)]
        assert not late
        return early, slots + [both(job) for job in p3q]

    ea, sl_a = make_slots([8 * i for i in range(2, 16)] + [256, 8, 0], P1_EARLY)
    eb, sl_b = make_slots([8 * i for i in range(16, 32)], P1_EARLY)
    paced([U(mm1s, 3, 2)], [(tok, ea, 0.35, 1), (tok_b, eb, 0.35 + 0.3 / len(eb), 1 + 0.3 / len(eb))], tail=100)
    wait(d5)

    su = [(p, tp) for tp in (3, 4) for p in range(4)]
    std = [U(mm1, (2 * q, 2 * q + 1), 10) for q in range(4)]
    std += [U(mm1, (p, p + 4), 2 * tp + o) for p, tp in su[NSB:] for o in range(2)]
    eu = [U(e_unit, q) for q in range(4)]
    std = [std[0], std[1], eu[0], std[2], eu[1], std[3], eu[2], eu[3]]
    strs = [U(mm1s, p, tp) for p, tp in su[:NSB]]
    tot = 512 * len(std) + 896 * SW * len(strs)
    na, nb = int(len(sl_a) * 512 * NH / (tot - BT)), int(len(sl_b) * 512 * NH / (tot - BT))
    wch = [w_chain(3, 0.1, 0.5), w_chain(4, 0.55, 0.95)]
    paced(std[0:NH], [(tok, sl_a[:na], 0, 1), (tok_b, sl_b[:nb], 0.5 / nb, 1 + 0.49 / nb)] + wch, tail=0)
    bu = [strs[0], std[6], strs[1], std[7]] + strs[2:]
    hb = 0.5 / len(sl_b[nb:])
    res_b = paced(bu, [(tok, sl_a[na:], 0, 1), (tok_b, sl_b[nb:], hb, 1 + hb), (tok_w, [U(w2_mini, n, 1) for n in range(40)], 0.03, 0.97)], tail=BT)

    vw[16 + z, 0, 0:8, :] = pltpu.bitcast(res_b[-1][1](VT), U32)
    pend = []
    zs = {}
    for s_lo in range(17):
        if s_lo < 16:
            pend.append(phase_c1(s_lo, zs[s_lo - DC - 1][0:4] if s_lo - DC - 1 >= 0 else None))
        if s_lo >= 1:
            sg = s_lo - 1
            zs[sg] = phase_c2(sg, zs[sg - DC][4:8] if sg - DC >= 0 else None, sg + DC < 16, *pend[sg])

    outs = []
    tok_act(pend[TOKC][0][0:8])
    for c, (r0, r1) in enumerate(MM2_CHUNKS):
        cps, m1, toks = mm2(r0, r1)
        outs += cps
        if r1 != 1024:
            tok_act(pltpu.bitcast(m1[0:8, 0:128], U32))
            jobs = gate_jobs(c + 1)
            for n, job in enumerate(jobs):
                tok_x(toks[n * (len(toks) - 4) // len(jobs)])
                job()
            gate2(c + 1)
    wait(outs)


@jax.jit
def pallas_gated_mix__spectral_gfnet__dense_activation_silu__prompt_kernel(A_x, A_w_r, A_w_i, B_x, B_w1, B_w2, gate_w):
    small, g = _consts()
    out = pl.pallas_call(
        _kernel,
        out_shape=jax.ShapeDtypeStruct((S, D), BF16),
        grid=(2,),
        in_specs=[pl.BlockSpec(memory_space=pl.ANY)] * 8,
        out_specs=pl.BlockSpec(memory_space=pl.ANY),
        scratch_shapes=[
            pltpu.VMEM((S // 2 + 8, D), U32),
            pltpu.VMEM((128, S), U32),
            pltpu.VMEM((128, S + 256), U32),
            pltpu.VMEM((1, S), BF16),
            pltpu.VMEM((1, S), BF16),
            pltpu.VMEM((16, S), BF16),
            pltpu.VMEM((16, S), BF16),
            pltpu.VMEM((FP // 2, D), U32),
            pltpu.VMEM((WS_END + 8, D), U32),
            pltpu.VMEM((D,), BF16),
            pltpu.VMEM((O_END, 128), U32),
            pltpu.VMEM((32, 64, 128), U32),
            pltpu.VMEM((18 * UB, 128), U32),
            pltpu.VMEM((16, 2, 152, 128), F32),
            pltpu.VMEM((16, 2, 152, 128), F32),
            pltpu.VMEM((17, 2, 272, 128), BF16),
            pltpu.VMEM((4 * AT + 32, 128), F32),
            pltpu.VMEM((8, S), F32),
            pltpu.VMEM((NF + 1, S + 16, 128), BF16),
            pltpu.VMEM((2, S + 8, 128), F32),
            pltpu.VMEM((24, 128), F32),
            pltpu.VMEM((S, D), F32),
            pltpu.VMEM((64, D), U32),
            pltpu.VMEM((S, D), BF16),
            *[pltpu.VMEM((11, 272, 128), BF16)] * 4,
            *[pltpu.VMEM((11, 144, 128), BF16)] * 5,
            pltpu.SemaphoreType.DMA((3,)),
        ],
        compiler_params=pltpu.CompilerParams(vmem_limit_bytes=100 * 1024 * 1024),
    )(A_x[0], A_w_r.T, A_w_i.T, B_w1.T, B_w2, gate_w, jnp.asarray(small), jnp.asarray(g))
    return out[None]
```
